```python
import jax
import jax.numpy as jnp

def _softmax(x, axis=-1):
    return jax.nn.softmax(x, axis=axis)

def _gelu(x):
    return jax.nn.gelu(x, approximate=True)

def _silu(x):
    return jax.nn.silu(x)

def _sigmoid(x):
    return jax.nn.sigmoid(x)

def _layernorm(x, axis=-1, eps=1e-05):
    m = jnp.mean(x, axis=axis, keepdims=True)
    v = jnp.var(x, axis=axis, keepdims=True)
    return (x - m) / jnp.sqrt(v + eps)

def _scatter_add(tgt, idx, src, axis=0):
    return tgt.at[idx].add(src)

def _segment_sum(src, seg, n):
    return jax.ops.segment_sum(src, seg, n)

class _Rng:

    def __init__(self, key):
        self._k = key

    def _next(self):
        self._k, sub = jax.random.split(self._k)
        return sub

    def normal(self, shape):
        return jax.random.normal(self._next(), shape, dtype=jnp.bfloat16)

    def randint(self, lo, hi, shape):
        return jax.random.randint(self._next(), shape, lo, hi, dtype=jnp.int32)

    def uniform(self, shape, lo=0.0, hi=1.0):
        return jax.random.uniform(self._next(), shape, jnp.bfloat16, lo, hi)

    def permutation(self, n):
        return jax.random.permutation(self._next(), n)
kernel_name = 'adaLN_cond__sliding_block_cached__dense_activation_mish__decode'

def setup_inputs():
    _rng = _Rng(jax.random.key(int.from_bytes(__import__("os").urandom(4), "little")))
    _w = lambda a: (lambda t: t.astype(jnp.bfloat16) if jnp.issubdtype(t.dtype, jnp.floating) else t)(jnp.asarray(a))

    def _A_setup():
        B, Sq, D = (1, 1, 640)
        Hq, Hkv, Sk, Dh = (32, 32, 32768, 192)
        assert Hq % Hkv == 0, (Hq, Hkv)
        return {'x': _w((lambda *s: _rng.normal(s) * 0.05)(B, Sq, D)), 'k_cache': _w((lambda *s: _rng.normal(s) * 0.05)(B, Hkv, Sk, Dh)), 'v_cache': _w((lambda *s: _rng.normal(s) * 0.05)(B, Hkv, Sk, Dh)), 'wq': _w((lambda *s: _rng.normal(s) * 0.05)(D, Hq * Dh) * D ** (-0.5)), 'wo': _w((lambda *s: _rng.normal(s) * 0.05)(Hq * Dh, D) * (Hq * Dh) ** (-0.5))}
    _A_in = _A_setup()

    def _B_setup():
        B, S, D, F = (1, 1, 640, 1536)
        return {'x': _w((lambda *s: _rng.normal(s) * 0.05)(B, S, D)), 'w1': _w((lambda *s: _rng.normal(s) * 0.05)(D, F) * D ** (-0.5)), 'b1': _w((lambda *s: _rng.normal(s) * 0.05)(F)), 'w2': _w((lambda *s: _rng.normal(s) * 0.05)(F, D) * F ** (-0.5))}
    _B_in = _B_setup()
    return {'A_x': _A_in['x'], 'A_k_cache': _A_in['k_cache'], 'A_v_cache': _A_in['v_cache'], 'A_wq': _A_in['wq'], 'A_wo': _A_in['wo'], 'B_x': _B_in['x'], 'B_w1': _B_in['w1'], 'B_b1': _B_in['b1'], 'B_w2': _B_in['w2'], 'c': _w((lambda *s: _rng.normal(s) * 0.05)(1, 640)), 'w_mod': _w((lambda *s: _rng.normal(s) * 0.05)(640, 6 * 640) * 640 ** (-0.5))}

def reference(A_x, A_k_cache, A_v_cache, A_wq, A_wo, B_x, B_w1, B_b1, B_w2, c, w_mod):

    def _A_ref(x, k_cache, v_cache, wq, wo):
        B, Sq, D = x.shape
        Hq, Dh = (32, 192)
        Hkv, Sk = (k_cache.shape[1], k_cache.shape[2])
        W = min(4096, max(256, Sk // 4))
        rep = Hq // Hkv
        q = (lambda x, *d: x.transpose(*d))((x @ wq).reshape(B, Sq, Hq, Dh), 0, 2, 1, 3)
        k = jnp.repeat(k_cache[:, :, Sk - W:, :], rep, axis=1)
        v = jnp.repeat(v_cache[:, :, Sk - W:, :], rep, axis=1)
        scores = jnp.einsum('bhqd,bhkd->bhqk', q, k) * Dh ** (-0.5)
        p = _softmax(scores, axis=-1)
        o = jnp.einsum('bhqk,bhkd->bhqd', p, v)
        return (lambda x, *d: x.transpose(*d))(o, 0, 2, 1, 3).reshape(B, Sq, Hq * Dh) @ wo

    def _B_ref(x, w1, b1, w2):
        h = jnp.einsum('bsd,df->bsf', x, w1) + b1
        sp = jnp.log1p(jnp.exp(-jnp.abs(h))) + jnp.where(h > 0, h, jnp.zeros_like(h))
        act = h * jnp.tanh(sp)
        return jnp.einsum('bsf,fd->bsd', act, w2)
    x = A_x
    mod = (_silu(c) @ w_mod).reshape(c.shape[0], 6, 1, -1)
    sa, ca, ga, sb, cb, gb = (mod[:, 0].copy(), mod[:, 1].copy(), mod[:, 2].copy(), mod[:, 3].copy(), mod[:, 4].copy(), mod[:, 5].copy())
    h = _layernorm(x, axis=-1) * (1 + ca) + sa
    x = x + ga * _A_ref(h, A_k_cache, A_v_cache, A_wq, A_wo)
    h = _layernorm(x, axis=-1) * (1 + cb) + sb
    x = x + gb * _B_ref(h, B_w1, B_b1, B_w2)
    return x
```

```python
import functools

import jax
import jax.numpy as jnp
from jax import lax
import jax.experimental.pallas as pl
import jax.experimental.pallas.tpu as pltpu

D, H, DH, F = 640, 32, 192, 1536
PAIR = 2 * DH
NPAIR = H // 2
LANE = 128
SUB = 8
PIECE = 8
F32, BF16 = jnp.float32, jnp.bfloat16

DEFAULT = dict(G=6, kvmode="fwd", jmod=36, jqo=64, j1=(20,), j2=20, look=80, lead=0, compute=True, bounds=True,
               w2_groups=((0, 6), (0, 4), (1, 4), (0, 2), (1, 4), (1, 2), (1, 2)), fence=True, tail_look=80, gather="stack")


def _layernorm(x, eps=1e-5):
    m = jnp.mean(x, axis=-1, keepdims=True)
    d = x - m
    v = jnp.mean(d * d, axis=-1, keepdims=True)
    return d / jnp.sqrt(v + eps)


def _mish(u):
    softplus = jnp.log1p(jnp.exp(-jnp.abs(u))) + jnp.where(u > 0, u, 0.0)
    return u * jnp.tanh(softplus)


def _dot(a, b):
    return jnp.dot(a, b, preferred_element_type=F32)


def _walk(lo, hi, jump):
    return [lo + i for o in range(jump) for i in range(o, hi - lo, jump)]


def _wait_all(buf, sem):
    pltpu.make_async_copy(buf, buf, sem).wait()


class _Stream:
    def __init__(self, q0, q1):
        self.order = []
        for i in range(0, max(len(q0), len(q1)), 2):
            self.order += [(cp, 0) for cp in q0[i:i + 2]] + [(cp, 1) for cp in q1[i:i + 2]]
        self.pos = 0

    def more(self, n):
        for cp, queue in self.order[self.pos:self.pos + n]:
            cp().start(priority=queue)
        self.pos += n

    def upto(self, n):
        self.more(max(n - self.pos, 0))

    def rest(self):
        self.upto(len(self.order))


def _kernel(x_hbm, k_hbm, v_hbm, wq_hbm, wo_hbm, w1_hbm, b1_hbm, w2_hbm, c_hbm, wmod_hbm, o_ref,
            x_v, c_v, b1_v, wmod_v, wq_v, wo_v, w1_v, w2_v, kv_v, q_s, s_s, m_s, o_s, att_s, mod_s,
            sem_w, sem_kv, sem_fence, *, window, cfg):
    nc = window // LANE
    c_first = k_hbm.shape[1] - nc
    half = nc // 2
    look = cfg["look"]
    compute = cfg["compute"]

    def mark(name):
        if cfg.get("marks"):
            with jax.named_scope("M_" + name):
                pl.delay(1)

    def fence():
        if cfg["fence"]:
            pl.semaphore_signal(sem_fence, 1)
            pl.semaphore_wait(sem_fence, 1)

    def flat(src, dst, sem, pieces):
        return [functools.partial(pltpu.make_async_copy, src.at[pl.ds(i * PIECE, PIECE)],
                                  dst.at[pl.ds(i * PIECE, PIECE)], sem) for i in pieces]

    def column(buf, ncol, j, row0, nrow):
        t0, n = row0 // SUB, nrow // SUB
        if cfg["gather"] == "stack":
            return jnp.stack([buf[(t0 + r) * ncol + j] for r in range(n)]).reshape(nrow, LANE)
        return buf[pl.ds(t0 * ncol + j, n, stride=ncol)].reshape(nrow, LANE)

    def kv_stream(src, p, h):
        rows, g = PAIR // SUB, cfg["G"]
        row0, slot = p * rows, (p % 2) * 2 + h
        lists = []
        for parity in range(2):
            mine = list(range(parity, rows, 2))
            out = []
            for i in range(0, len(mine), g):
                rs = mine[i:i + g]
                for n, c in enumerate(range(0, half, PIECE)):
                    o = rs if n % 2 == 0 or cfg["kvmode"] == "fwd" else rs[::-1] if cfg["kvmode"] == "zig" else rs[1:] + rs[:1]
                    out += [functools.partial(
                        pltpu.make_async_copy,
                        src.at[row0 + r, pl.ds(c_first + h * half + c, PIECE)],
                        kv_v.at[slot, pl.ds(c, PIECE), pl.ds(r * SUB, SUB), :], sem_kv.at[slot]) for r in o]
            lists.append(out)
        return _Stream(*lists)

    s_c, s_x, s_b1, s_wmod, s_wq, s_wo, s_w1 = range(7)
    s_w2 = s_w1 + len(cfg["j1"])
    small = [functools.partial(pltpu.make_async_copy, s, d, sem_w.at[i])
             for i, s, d in ((s_c, c_hbm, c_v), (s_x, x_hbm, x_v), (s_b1, b1_hbm, b1_v))]

    n = wmod_hbm.shape[0] // PIECE
    st = _Stream(flat(wmod_hbm, wmod_v, sem_w.at[s_wmod], _walk(0, n // 2, cfg["jmod"])),
                 flat(wmod_hbm, wmod_v, sem_w.at[s_wmod], _walk(n // 2, n, cfg["jmod"])))
    st.more(4)
    for cp in small:
        cp().start()
    st.rest()
    fence()

    mark("wmod")
    n = wo_hbm.shape[0] // PIECE
    per_row = H * DH // LANE // PIECE
    st = _Stream([functools.partial(pltpu.make_async_copy, wq_hbm.at[pl.ds(i * PIECE, PIECE)],
                                    wq_v.at[pl.ds(i % per_row * PIECE, PIECE), pl.ds(i // per_row * SUB, SUB), :],
                                    sem_w.at[s_wq]) for i in _walk(0, n, cfg["jqo"])],
                 flat(wo_hbm, wo_v, sem_w.at[s_wo], _walk(0, n, cfg["jqo"])))
    st.more(look)
    for cp in small:
        cp().wait()
    _wait_all(wmod_v, sem_w.at[s_wmod])
    nd = D // LANE
    if compute:
        cf = c_v[...].astype(F32)
        silu_c = jnp.broadcast_to(cf * jax.nn.sigmoid(cf), (8, D)).astype(BF16)
        for j in range(6 * nd):
            mod_s[j // nd, :, j % nd * LANE:(j % nd + 1) * LANE] = _dot(silu_c, column(wmod_v, 6 * nd, j, 0, D))
            st.more(8)
        x0 = jnp.broadcast_to(x_v[...].astype(F32), (8, D))
        h1 = (_layernorm(x0) * (1.0 + mod_s[1]) + mod_s[0]).astype(BF16)
    st.rest()
    fence()

    mark("wqo")
    row = lax.broadcasted_iota(jnp.int32, (8, PAIR), 0)
    col = lax.broadcasted_iota(jnp.int32, (8, PAIR), 1)
    own = jnp.logical_or(jnp.logical_and(row == 0, col < DH), jnp.logical_and(row == 1, col >= DH))

    def query(p, st, step):
        if not compute:
            return
        parts = []
        for j in range(PAIR // LANE):
            parts.append(_dot(h1, wq_v[p * (PAIR // LANE) + j]))
            st.more(step)
        q_s[p] = jnp.where(own, jnp.concatenate(parts, axis=1), 0.0)

    def scores(p, h, st, step):
        slot = (p % 2) * 2 + h
        _wait_all(kv_v.at[slot], sem_kv.at[slot])
        if not compute:
            return
        q = q_s[p].astype(BF16)
        m = None if h == 0 else m_s[p]
        for c in range(half):
            s = _dot(q, kv_v[slot, c]) * DH ** -0.5
            s_s[p, h * half + c] = s
            m = s if m is None else jnp.maximum(m, s)
            st.more(step)
        m_s[p] = m

    def values(p, h, st, step, carry):
        slot = (p % 2) * 2 + h
        _wait_all(kv_v.at[slot], sem_kv.at[slot])
        if not compute:
            return None
        if h == 0:
            carry = (jnp.max(m_s[p], axis=-1, keepdims=True), jnp.zeros((8, LANE), F32), jnp.zeros((8, PAIR), F32))
        m, l, acc = carry
        for c in range(half):
            e = jnp.exp(s_s[p, h * half + c] - m)
            l += e
            acc += lax.dot_general(e.astype(BF16), kv_v[slot, c], (((1,), (1,)), ((), ())),
                                   preferred_element_type=F32)
            st.more(step)
        if h == 0:
            return m, l, acc
        return jnp.where(own, acc / jnp.sum(l, axis=-1, keepdims=True), 0.0)

    def project(p, o, st, step):
        if not compute:
            return 0.0
        o = o.astype(BF16)
        parts = []
        for j in range(nd):
            parts.append(_dot(o, column(wo_v, nd, j, p * PAIR, PAIR)))
            st.more(step)
        return jnp.concatenate(parts, axis=1)

    st = kv_stream(k_hbm, 0, 0)
    st.more(look)
    _wait_all(wq_v, sem_w.at[s_wq])
    _wait_all(wo_v, sem_w.at[s_wo])
    st.rest()
    st = kv_stream(k_hbm, 0, 1)
    query(0, st, 8)
    st.rest()

    def k_body(p, carry):
        st = kv_stream(k_hbm, p, 0)
        scores(p - 1, 0, st, 6)
        st.rest()
        st = kv_stream(k_hbm, p, 1)
        scores(p - 1, 1, st, 5)
        query(p, st, 5)
        st.rest()
        return carry

    mark("k0")
    lax.fori_loop(1, NPAIR, k_body, 0)
    mark("k")

    for h in range(2):
        st = kv_stream(v_hbm, 0, h)
        scores(NPAIR - 1, h, st, 6)
        st.rest()
    if compute:
        o_s[...] = jnp.zeros(o_s.shape, F32)
        att_s[...] = jnp.zeros(att_s.shape, F32)

    def v_body(p, carry):
        st = kv_stream(v_hbm, p, 0)
        if compute:
            att_s[...] += project(jnp.maximum(p - 2, 0), o_s[...], st, 3)
        c = values(p - 1, 0, st, 5, None)
        st.rest()
        st = kv_stream(v_hbm, p, 1)
        o = values(p - 1, 1, st, 6, c)
        if compute:
            o_s[...] = o
        st.rest()
        return carry

    mark("v0")
    lax.fori_loop(1, NPAIR, v_body, 0)
    mark("v")

    n1 = w1_hbm.shape[0] // PIECE
    parts1 = len(cfg["j1"])
    q0, q1, ends = [], [], []
    for i, jump in enumerate(cfg["j1"]):
        lo, hi = i * n1 // parts1, (i + 1) * n1 // parts1
        mid = (lo + hi) // 2
        q0 += flat(w1_hbm, w1_v, sem_w.at[s_w1 + i], _walk(lo, mid, jump))
        q1 += flat(w1_hbm, w1_v, sem_w.at[s_w1 + i], _walk(mid, hi, jump))
        ends.append(len(q0) + len(q1))
    unit = 64
    per = unit // SUB * nd // PIECE
    nb = F // LANE
    nxt = [0, sum(k for queue, k in cfg["w2_groups"] if queue == 0)]
    groups = []
    for i, (queue, k) in enumerate(cfg["w2_groups"]):
        b = nxt[queue]
        (q0, q1)[queue].extend(flat(w2_hbm, w2_v, sem_w.at[s_w2 + i], _walk(b * per, (b + k) * per, cfg["j2"])))
        groups.append((b, b + k))
        nxt[queue] += k
    assert nxt[1] * unit == F
    st = _Stream(q0, q1)

    att = project(NPAIR - 2, o_s[...], st, 3) if compute else 0.0
    c = values(NPAIR - 1, 0, st, 4, None)
    st.upto(look)
    o = values(NPAIR - 1, 1, st, 2, c)
    att = att + project(NPAIR - 1, o, st, 2)
    if compute:
        att = jnp.broadcast_to(jnp.sum(att_s[...] + att, axis=0, keepdims=True), (8, D))
        x1 = x0 + mod_s[2] * att
        h2 = (_layernorm(x1) * (1.0 + mod_s[4]) + mod_s[3]).astype(BF16)
        b1 = b1_v[...].astype(F32)
        u = [jnp.broadcast_to(b1[j:j + 1, :], (8, LANE)) for j in range(nb)]
    rows = D // parts1
    mark("h2")
    for i in range(parts1):
        st.upto(ends[i] + cfg["tail_look"])
        _wait_all(w1_v.at[pl.ds(i * n1 // parts1 * PIECE, n1 // parts1 * PIECE)], sem_w.at[s_w1 + i])
        if compute:
            for j in range(nb):
                u[j] += _dot(h2[:, i * rows:(i + 1) * rows], column(w1_v, nb, j, i * rows, rows))
                st.more(2)
    st.rest()
    mark("issued")
    if compute:
        act = _mish(jnp.concatenate(u, axis=1)).astype(BF16)
        y = [jnp.zeros((8, LANE), F32)] * nd
    for i, (b0, b1_) in enumerate(groups):
        _wait_all(w2_v.at[pl.ds(b0 * per * PIECE, (b1_ - b0) * per * PIECE)], sem_w.at[s_w2 + i])
        mark(f"w2_{i}")
        if compute:
            a = act[:, b0 * unit:b1_ * unit]
            y = [y[j] + _dot(a, column(w2_v, nd, j, b0 * unit, (b1_ - b0) * unit)) for j in range(nd)]
    if compute:
        o_ref[...] = (x1 + mod_s[5] * jnp.concatenate(y, axis=1))[0:1].astype(o_ref.dtype)
    else:
        o_ref[...] = jnp.zeros(o_ref.shape, o_ref.dtype)


def _tiles(a):
    r, c = a.shape
    return a.reshape(r // SUB, SUB, c // LANE, LANE).transpose(0, 2, 1, 3)


def _flat(a):
    return _tiles(a).reshape(-1, SUB, LANE)


def make(**over):
    cfg = dict(DEFAULT)
    cfg.update(over)

    def fn(A_x, A_k_cache, A_v_cache, A_wq, A_wo, B_x, B_w1, B_b1, B_w2, c, w_mod):
        del B_x
        sk = A_k_cache.shape[2]
        window = min(4096, max(256, sk // 4))
        nc = window // LANE
        kt = _tiles(jnp.swapaxes(A_k_cache, 2, 3).reshape(H * DH, sk))
        vt = _tiles(jnp.swapaxes(A_v_cache, 2, 3).reshape(H * DH, sk))
        wmod, wo, w1, w2 = _flat(w_mod), _flat(A_wo), _flat(B_w1), _flat(B_w2)
        hbm = pl.BlockSpec(memory_space=pltpu.HBM)
        out = pl.pallas_call(
            functools.partial(_kernel, window=window, cfg=cfg),
            out_shape=jax.ShapeDtypeStruct((1, D), A_x.dtype),
            in_specs=[hbm] * 10,
            out_specs=pl.BlockSpec(memory_space=pltpu.VMEM),
            scratch_shapes=[
                pltpu.VMEM((1, D), BF16), pltpu.VMEM((1, D), BF16), pltpu.VMEM((F // LANE, LANE), BF16),
                pltpu.VMEM(wmod.shape, BF16),
                pltpu.VMEM((H * DH // LANE, D, LANE), BF16),
                pltpu.VMEM(wo.shape, BF16), pltpu.VMEM(w1.shape, BF16), pltpu.VMEM(w2.shape, BF16),
                pltpu.VMEM((4, nc // 2, PAIR, LANE), BF16),
                pltpu.VMEM((NPAIR, 8, PAIR), F32),
                pltpu.VMEM((NPAIR, nc, 8, LANE), F32),
                pltpu.VMEM((NPAIR, 8, LANE), F32),
                pltpu.VMEM((8, PAIR), F32),
                pltpu.VMEM((8, D), F32),
                pltpu.VMEM((6, 8, D), F32),
                pltpu.SemaphoreType.DMA((6 + len(cfg["j1"]) + len(cfg["w2_groups"]),)),
                pltpu.SemaphoreType.DMA((4,)),
                pltpu.SemaphoreType.REGULAR,
            ],
            compiler_params=pltpu.CompilerParams(vmem_limit_bytes=64 * 2**20, disable_semaphore_checks=True,
                                                 disable_bounds_checks=not cfg["bounds"], flags=cfg.get("flags")),
            name="adaln_attn_mlp_decode",
        )(A_x.reshape(1, D), kt, vt, _flat(A_wq), wo, w1, B_b1.reshape(F // LANE, LANE), w2, c, wmod)
        return out.reshape(A_x.shape)
    return fn


pallas_adaLN_cond__sliding_block_cached__dense_activation_mish__decode_kernel = jax.jit(make())
```

```python
import functools

import jax
import jax.numpy as jnp
from jax import lax
import jax.experimental.pallas as pl
import jax.experimental.pallas.tpu as pltpu

D, H, DH, F = 640, 32, 192, 1536
PAIR = 2 * DH
NPAIR = H // 2
LANE = 128
SUB = 8
PIECE = 8
F32, BF16 = jnp.float32, jnp.bfloat16

DEFAULT = dict(G=6, kvmode="fwd", kvwhole=False, A=(64, 2, 22), j2=20, look=104, compute=True, bounds=True,
               w2_groups=((0, 8), (1, 6), (0, 4), (1, 3), (1, 2), (1, 1)), fence=True, tail=(30, 96, 112, 130),
               gather="stack", ramp="10111" * 9, w1_late=32, vpu=2, unit=64)


def _layernorm(x, eps=1e-5):
    m = jnp.mean(x, axis=-1, keepdims=True)
    d = x - m
    v = jnp.mean(d * d, axis=-1, keepdims=True)
    return d / jnp.sqrt(v + eps)


def _mish(u):
    softplus = jnp.log1p(jnp.exp(-jnp.abs(u))) + jnp.where(u > 0, u, 0.0)
    return u * jnp.tanh(softplus)


def _dot(a, b):
    return jnp.dot(a, b, preferred_element_type=F32)


def _walk(items, jump, k=1, group=10**9):
    out = []
    for o in range(0, jump, k):
        starts = list(range(o, len(items), jump))
        for g in range(0, len(starts), group):
            for c in range(min(k, jump - o)):
                out += [items[r + c] for r in starts[g:g + group] if r + c < len(items)]
    assert len(out) == len(items)
    return out


def _wait_all(buf, sem):
    pltpu.make_async_copy(buf, buf, sem).wait()


class _Stream:
    def __init__(self, q0, q1, ramp=""):
        lists, pos = (q0, q1), [0, 0]
        self.order = []
        for queue in map(int, ramp):
            self.order.append((lists[queue][pos[queue]], queue))
            pos[queue] += 1
        while len(self.order) < len(q0) + len(q1):
            for queue in (0, 1):
                self.order += [(cp, queue) for cp in lists[queue][pos[queue]:pos[queue] + 2]]
                pos[queue] += 2
        self.pos = 0

    def more(self, n):
        for cp, queue in self.order[self.pos:self.pos + n]:
            cp().start(priority=queue)
        self.pos += n

    def upto(self, n):
        self.more(max(n - self.pos, 0))

    def rest(self):
        self.upto(len(self.order))


def _kernel(x_hbm, k_hbm, v_hbm, wq_hbm, wo_hbm, w1_hbm, b1_hbm, w2_hbm, c_hbm, wmod_hbm, o_ref,
            x_v, c_v, b1_v, wmod_v, wq_v, wo_v, w1_v, w2_v, kv_v, q_s, s_s, m_s, o_s, att_s, mod_s,
            sem_w, sem_kv, sem_fence, *, window, cfg):
    nc = window // LANE
    c_first = k_hbm.shape[1] - nc
    half = nc // 2
    look = cfg["look"]
    compute = cfg["compute"]

    def mark(name):
        if cfg.get("marks"):
            with jax.named_scope("M_" + name):
                pl.delay(1)

    def fence():
        if cfg["fence"]:
            pl.semaphore_signal(sem_fence, 1)
            pl.semaphore_wait(sem_fence, 1)

    def flat(src, dst, sem):
        return [functools.partial(pltpu.make_async_copy, src.at[pl.ds(i, PIECE)], dst.at[pl.ds(i, PIECE)], sem)
                for i in range(0, src.shape[0], PIECE)]

    def column(buf, ncol, j, row0, nrow):
        t0, n = row0 // SUB, nrow // SUB
        if cfg["gather"] == "stack":
            return jnp.stack([buf[(t0 + r) * ncol + j] for r in range(n)]).reshape(nrow, LANE)
        return buf[pl.ds(t0 * ncol + j, n, stride=ncol)].reshape(nrow, LANE)

    def kv_lists(src, p, h):
        rows, g = PAIR // SUB, cfg["G"]
        row0, slot = p * rows, (p % 2) * 2 + h
        lists = []
        for parity in range(2):
            mine = list(range(parity, rows, 2))
            out = []
            for i in range(0, len(mine), g):
                rs = mine[i:i + g]
                for n, c in enumerate(range(0, half, PIECE)):
                    o = rs if n % 2 == 0 or cfg["kvmode"] == "fwd" else rs[::-1] if cfg["kvmode"] == "zig" else rs[1:] + rs[:1]
                    out.append([functools.partial(
                        pltpu.make_async_copy,
                        src.at[row0 + r, pl.ds(c_first + h * half + c, PIECE)],
                        kv_v.at[slot, pl.ds(c, PIECE), pl.ds(r * SUB, SUB), :], sem_kv.at[slot]) for r in o])
            lists.append(out)
        return lists

    def kv_stream(src, p):
        a, b = kv_lists(src, p, 0), kv_lists(src, p, 1)
        n = cfg["kvwhole"] or len(a[0])
        return _Stream(*[[cp for i in range(0, len(a[q]), n) for part in a[q][i:i + n] + b[q][i:i + n] for cp in part]
                         for q in range(2)])

    s_c, s_x, s_b1, s_wmod, s_wq, s_wo, s_w1, s_w2 = range(8)
    small = [functools.partial(pltpu.make_async_copy, s, d, sem_w.at[i])
             for i, s, d in ((s_c, c_hbm, c_v), (s_x, x_hbm, x_v), (s_b1, b1_hbm, b1_v))]

    per_row = H * DH // LANE // PIECE
    w1_copies = flat(w1_hbm, w1_v, sem_w.at[s_w1])
    early = len(w1_copies) - cfg["w1_late"]
    weights = (flat(wmod_hbm, wmod_v, sem_w.at[s_wmod]) + w1_copies[:early] + flat(wo_hbm, wo_v, sem_w.at[s_wo])
               + [functools.partial(pltpu.make_async_copy, wq_hbm.at[pl.ds(i * PIECE, PIECE)],
                                    wq_v.at[pl.ds(i % per_row * PIECE, PIECE), pl.ds(i // per_row * SUB, SUB), :],
                                    sem_w.at[s_wq]) for i in range(wq_hbm.shape[0] // PIECE)])
    ramp = cfg["ramp"] or ""
    n = (len(weights) + ramp.count("0") - ramp.count("1")) // 2
    st = _Stream(_walk(weights[:n], *cfg["A"]), _walk(weights[n:], *cfg["A"]), ramp)
    st.more(cfg.get("small_at", 4))
    fence()
    for cp in small:
        cp().start()
    while st.pos < len(st.order):
        fence()
        st.more(cfg.get("fence_every", 4))
    fence()
    mark("w")

    row = lax.broadcasted_iota(jnp.int32, (8, PAIR), 0)
    col = lax.broadcasted_iota(jnp.int32, (8, PAIR), 1)
    own = jnp.logical_or(jnp.logical_and(row == 0, col < DH), jnp.logical_and(row == 1, col >= DH))
    nd = D // LANE

    def query(p, st, step):
        if not compute:
            return
        parts = []
        for j in range(PAIR // LANE):
            parts.append(_dot(h1, wq_v[p * (PAIR // LANE) + j]))
            st.more(step)
        q_s[p] = jnp.where(own, jnp.concatenate(parts, axis=1), 0.0)

    def scores(p, h, st, step):
        slot = (p % 2) * 2 + h
        _wait_all(kv_v.at[slot], sem_kv.at[slot])
        if not compute:
            return
        q = q_s[p].astype(BF16)
        m = None if h == 0 else m_s[p]
        for c in range(half):
            s = _dot(q, kv_v[slot, c]) * DH ** -0.5
            s_s[p, h * half + c] = s
            m = s if m is None else jnp.maximum(m, s)
            st.more(step)
        m_s[p] = m

    def values(p, h, st, step, carry):
        slot = (p % 2) * 2 + h
        _wait_all(kv_v.at[slot], sem_kv.at[slot])
        if not compute:
            return None
        if h == 0:
            carry = (jnp.max(m_s[p], axis=-1, keepdims=True), jnp.zeros((8, LANE), F32), jnp.zeros((8, PAIR), F32))
        m, l, acc = carry
        for c in range(half):
            e = jnp.exp(s_s[p, h * half + c] - m)
            l += e
            acc += lax.dot_general(e.astype(BF16), kv_v[slot, c], (((1,), (1,)), ((), ())),
                                   preferred_element_type=F32)
            st.more(step)
        if h == 0:
            return m, l, acc
        return jnp.where(own, acc / jnp.sum(l, axis=-1, keepdims=True), 0.0)

    def project(p, o, st, step):
        if not compute:
            return 0.0
        o = o.astype(BF16)
        parts = []
        for j in range(nd):
            parts.append(_dot(o, column(wo_v, nd, j, p * PAIR, PAIR)))
            st.more(step)
        return jnp.concatenate(parts, axis=1)

    st = kv_stream(k_hbm, 0)
    st.more(look)
    for cp in small:
        cp().wait()
    _wait_all(wmod_v, sem_w.at[s_wmod])
    _wait_all(wq_v, sem_w.at[s_wq])
    _wait_all(wo_v, sem_w.at[s_wo])
    if compute:
        cf = c_v[...].astype(F32)
        silu_c = jnp.broadcast_to(cf * jax.nn.sigmoid(cf), (8, D)).astype(BF16)
        for j in range(6 * nd):
            mod_s[j // nd, :, j % nd * LANE:(j % nd + 1) * LANE] = _dot(silu_c, column(wmod_v, 6 * nd, j, 0, D))
            st.more(2)
        x0 = jnp.broadcast_to(x_v[...].astype(F32), (8, D))
        h1 = (_layernorm(x0) * (1.0 + mod_s[1]) + mod_s[0]).astype(BF16)
    query(0, st, 4)
    st.rest()
    sl = cfg.get("slook", 0)

    def k_body(p, carry):
        st = kv_stream(k_hbm, p)
        st.more(sl)
        scores(p - 1, 0, st, 5 if not sl else 2)
        st.upto(96)
        scores(p - 1, 1, st, 5)
        query(p, st, 5)
        st.rest()
        return carry

    mark("k0")
    lax.fori_loop(1, NPAIR, k_body, 0)
    mark("k")

    st = kv_stream(v_hbm, 0)
    st.more(sl)
    scores(NPAIR - 1, 0, st, 5 if not sl else 2)
    st.upto(96)
    scores(NPAIR - 1, 1, st, 5)
    st.rest()
    if compute:
        o_s[...] = jnp.zeros(o_s.shape, F32)
        att_s[...] = jnp.zeros(att_s.shape, F32)

    def v_body(p, carry):
        st = kv_stream(v_hbm, p)
        if compute:
            att_s[...] += project(jnp.maximum(p - 2, 0), o_s[...], st, 3)
        st.upto(sl)
        c = values(p - 1, 0, st, 5 if not sl else 2, None)
        st.upto(96)
        o = values(p - 1, 1, st, 5, c)
        if compute:
            o_s[...] = o
        st.rest()
        return carry

    mark("v0")
    lax.fori_loop(1, NPAIR, v_body, 0)
    mark("v")

    late = w1_copies[early:]
    q0, q1 = _walk(late[:len(late) // 2], cfg["j2"]), _walk(late[len(late) // 2:], cfg["j2"])
    unit = cfg["unit"]
    per = unit // SUB * nd // PIECE
    nb = F // LANE
    nxt = [0, sum(k for queue, k in cfg["w2_groups"] if queue == 0)]
    groups = []
    for i, (queue, k) in enumerate(cfg["w2_groups"]):
        b = nxt[queue]
        (q0, q1)[queue].extend(_walk(flat(w2_hbm, w2_v, sem_w.at[s_w2 + i])[b * per:(b + k) * per], cfg["j2"]))
        groups.append((b, b + k))
        nxt[queue] += k
    assert nxt[1] * unit == F
    st = _Stream(q0, q1)

    t0, t1, t2, t3 = cfg["tail"]
    st.upto(t0)
    fence()
    att = project(NPAIR - 2, o_s[...], st, 0) if compute else 0.0
    c = values(NPAIR - 1, 0, st, 0, None)
    fence()
    st.upto(t1)
    mark("pv")
    o = values(NPAIR - 1, 1, st, 0, c)
    fence()
    st.upto(t2)
    fence()
    att = att + project(NPAIR - 1, o, st, 0)
    if compute:
        att = jnp.broadcast_to(jnp.sum(att_s[...] + att, axis=0, keepdims=True), (8, D))
        x1 = x0 + mod_s[2] * att
        h2 = (_layernorm(x1) * (1.0 + mod_s[4]) + mod_s[3]).astype(BF16)
        b1 = b1_v[...].astype(F32)
    st.upto(t3)
    mark("h2")
    _wait_all(w1_v, sem_w.at[s_w1])
    if compute:
        u = [jnp.broadcast_to(b1[j:j + 1, :], (8, LANE)) + _dot(h2, column(w1_v, nb, j, 0, D)) for j in range(nb)]
        act = _mish(jnp.concatenate(u, axis=1)).astype(BF16)
        y = [jnp.zeros((8, LANE), F32)] * nd
    fence()
    st.rest()
    nv = cfg["vpu"]
    if compute:
        scale = {}
        for b0, b1_ in groups[len(groups) - nv:]:
            for t in range(b0 * unit // LANE, -(-b1_ * unit // LANE)):
                scale[t] = jnp.broadcast_to(act[0:1, t * LANE:(t + 1) * LANE].astype(F32), (LANE, LANE)).T
        part = [None] * nd
    for i, (b0, b1_) in enumerate(groups):
        _wait_all(w2_v.at[pl.ds(b0 * per * PIECE, (b1_ - b0) * per * PIECE)], sem_w.at[s_w2 + i])
        mark(f"w2_{i}")
        if not compute:
            continue
        if i < len(groups) - nv:
            a = act[:, b0 * unit:b1_ * unit]
            y = [y[j] + _dot(a, column(w2_v, nd, j, b0 * unit, (b1_ - b0) * unit)) for j in range(nd)]
            continue
        for r in range(b0 * unit, b1_ * unit, SUB):
            a = scale[r // LANE][r % LANE:r % LANE + SUB]
            for j in range(nd):
                t = w2_v[r // SUB * nd + j].astype(F32) * a
                part[j] = t if part[j] is None else part[j] + t
    if compute:
        out = x1 + mod_s[5] * jnp.concatenate(y, axis=1)
        if nv:
            out = out[0:1] + mod_s[5, 0:1] * jnp.sum(jnp.concatenate(part, axis=1), axis=0, keepdims=True)
        o_ref[...] = out[0:1].astype(o_ref.dtype)
    else:
        o_ref[...] = jnp.zeros(o_ref.shape, o_ref.dtype)


def _tiles(a):
    r, c = a.shape
    return a.reshape(r // SUB, SUB, c // LANE, LANE).transpose(0, 2, 1, 3)


def _flat(a):
    return _tiles(a).reshape(-1, SUB, LANE)


def make(**over):
    cfg = dict(DEFAULT)
    cfg.update(over)

    def fn(A_x, A_k_cache, A_v_cache, A_wq, A_wo, B_x, B_w1, B_b1, B_w2, c, w_mod):
        del B_x
        sk = A_k_cache.shape[2]
        window = min(4096, max(256, sk // 4))
        nc = window // LANE
        kt = _tiles(jnp.swapaxes(A_k_cache, 2, 3).reshape(H * DH, sk))
        vt = _tiles(jnp.swapaxes(A_v_cache, 2, 3).reshape(H * DH, sk))
        wmod, wo, w1, w2 = _flat(w_mod), _flat(A_wo), _flat(B_w1), _flat(B_w2)
        hbm = pl.BlockSpec(memory_space=pltpu.HBM)
        out = pl.pallas_call(
            functools.partial(_kernel, window=window, cfg=cfg),
            out_shape=jax.ShapeDtypeStruct((1, D), A_x.dtype),
            in_specs=[hbm] * 10,
            out_specs=pl.BlockSpec(memory_space=pltpu.VMEM),
            scratch_shapes=[
                pltpu.VMEM((1, D), BF16), pltpu.VMEM((1, D), BF16), pltpu.VMEM((F // LANE, LANE), BF16),
                pltpu.VMEM(wmod.shape, BF16),
                pltpu.VMEM((H * DH // LANE, D, LANE), BF16),
                pltpu.VMEM(wo.shape, BF16), pltpu.VMEM(w1.shape, BF16), pltpu.VMEM(w2.shape, BF16),
                pltpu.VMEM((4, nc // 2, PAIR, LANE), BF16),
                pltpu.VMEM((NPAIR, 8, PAIR), F32),
                pltpu.VMEM((NPAIR, nc, 8, LANE), F32),
                pltpu.VMEM((NPAIR, 8, LANE), F32),
                pltpu.VMEM((8, PAIR), F32),
                pltpu.VMEM((8, D), F32),
                pltpu.VMEM((6, 8, D), F32),
                pltpu.SemaphoreType.DMA((7 + len(cfg["w2_groups"]),)),
                pltpu.SemaphoreType.DMA((4,)),
                pltpu.SemaphoreType.REGULAR,
            ],
            compiler_params=pltpu.CompilerParams(vmem_limit_bytes=64 * 2**20, disable_semaphore_checks=True,
                                                 disable_bounds_checks=not cfg["bounds"], flags=cfg.get("flags")),
            name="adaln_attn_mlp_decode",
        )(A_x.reshape(1, D), kt, vt, _flat(A_wq), wo, w1, B_b1.reshape(F // LANE, LANE), w2, c, wmod)
        return out.reshape(A_x.shape)
    return fn


pallas_adaLN_cond__sliding_block_cached__dense_activation_mish__decode_kernel = jax.jit(make())
```

```python
import functools

import jax
import jax.numpy as jnp
from jax import lax
import jax.experimental.pallas as pl
import jax.experimental.pallas.tpu as pltpu

D, H, DH, F = 640, 32, 192, 1536
PAIR = 2 * DH
NPAIR = H // 2
LANE = 128
SUB = 8
PIECE = 8
F32, BF16 = jnp.float32, jnp.bfloat16

DEFAULT = dict(G=6, kvmode="fwd", kvwhole=False, AG=11, j2=20, look=64, compute=True, bounds=False,
               w2_groups=((0, ((0, 4), (8, 12))), (1, ((12, 16), (20, 22))), (0, ((4, 8),)), (1, ((22, 24), (16, 17))), (1, ((17, 19),)), (1, ((19, 20),))), fence=True, tail=(30, 96, 114, 134),
               gather="stack", skv=(2, 2), sa=(2, 2), st=(1, 1), modstep=3, modfence=5, ramp="10111" * 5, w1_late=32, vpu=2, unit=64)


def _layernorm(x, eps=1e-5):
    m = jnp.mean(x, axis=-1, keepdims=True)
    d = x - m
    v = jnp.mean(d * d, axis=-1, keepdims=True)
    return d / jnp.sqrt(v + eps)


def _mish(u):
    softplus = jnp.log1p(jnp.exp(-jnp.abs(u))) + jnp.where(u > 0, u, 0.0)
    return u * jnp.tanh(softplus)


def _dot(a, b):
    return jnp.dot(a, b, preferred_element_type=F32)


def _walk(items, jump, k=1, group=10**9):
    out = []
    for o in range(0, jump, k):
        starts = list(range(o, len(items), jump))
        for g in range(0, len(starts), group):
            for c in range(min(k, jump - o)):
                out += [items[r + c] for r in starts[g:g + group] if r + c < len(items)]
    assert len(out) == len(items)
    return out


def _wait_all(buf, sem):
    pltpu.make_async_copy(buf, buf, sem).wait()


class _Stream:
    def __init__(self, q0, q1, split, ramp=""):
        lists, pos = (q0, q1), [0, 0]
        self.order = []
        self.split = split
        for queue in map(int, ramp):
            self.order.append((lists[queue][pos[queue]], queue))
            pos[queue] += 1
        while len(self.order) < len(q0) + len(q1):
            for queue in (0, 1):
                self.order += [(cp, queue) for cp in lists[queue][pos[queue]:pos[queue] + 2]]
                pos[queue] += 2
        self.pos = 0

    def more(self, n):
        for cp, queue in self.order[self.pos:self.pos + n]:
            k = PIECE // self.split[queue]
            for o in range(0, PIECE, k):
                cp(o, k).start(priority=queue)
        self.pos += n

    def upto(self, n):
        self.more(max(n - self.pos, 0))

    def rest(self):
        self.upto(len(self.order))


def _kernel(x_hbm, k_hbm, v_hbm, wq_hbm, wo_hbm, w1_hbm, b1_hbm, w2_hbm, c_hbm, wmod_hbm, o_ref,
            x_v, c_v, b1_v, wmod_v, wq_v, wo_v, w1_v, w2_v, kv_v, q_s, s_s, m_s, o_s, att_s, mod_s,
            sem_w, sem_kv, sem_fence, *, window, cfg):
    nc = window // LANE
    c_first = k_hbm.shape[1] - nc
    half = nc // 2
    look = cfg["look"]
    compute = cfg["compute"]

    def mark(name):
        if cfg.get("marks"):
            with jax.named_scope("M_" + name):
                pl.delay(1)

    def fence():
        if cfg["fence"]:
            pl.semaphore_signal(sem_fence, 1)
            pl.semaphore_wait(sem_fence, 1)

    def flat(src, dst, sem):
        return [lambda o, k, i=i: pltpu.make_async_copy(src.at[pl.ds(i + o, k)], dst.at[pl.ds(i + o, k)], sem)
                for i in range(0, src.shape[0], PIECE)]

    def column(buf, ncol, j, row0, nrow):
        t0, n = row0 // SUB, nrow // SUB
        if cfg["gather"] == "stack":
            return jnp.stack([buf[(t0 + r) * ncol + j] for r in range(n)]).reshape(nrow, LANE)
        return buf[pl.ds(t0 * ncol + j, n, stride=ncol)].reshape(nrow, LANE)

    def kv_lists(src, p, h):
        rows, g = PAIR // SUB, cfg["G"]
        row0, slot = p * rows, (p % 2) * 2 + h
        lists = []
        for parity in range(2):
            mine = list(range(parity, rows, 2))
            out = []
            for i in range(0, len(mine), g):
                rs = mine[i:i + g]
                for n, c in enumerate(range(0, half, PIECE)):
                    o = rs if n % 2 == 0 or cfg["kvmode"] == "fwd" else rs[::-1] if cfg["kvmode"] == "zig" else rs[1:] + rs[:1]
                    out.append([lambda o, k, r=r, c=c: pltpu.make_async_copy(
                        src.at[row0 + r, pl.ds(c_first + h * half + c + o, k)],
                        kv_v.at[slot, pl.ds(c + o, k), pl.ds(r * SUB, SUB), :], sem_kv.at[slot]) for r in o])
            lists.append(out)
        return lists

    def kv_stream(src, p):
        a, b = kv_lists(src, p, 0), kv_lists(src, p, 1)
        n = cfg["kvwhole"] or len(a[0])
        return _Stream(*[[cp for i in range(0, len(a[q]), n) for part in a[q][i:i + n] + b[q][i:i + n] for cp in part]
                         for q in range(2)], cfg["skv"])

    s_c, s_x, s_b1, s_wmod, s_wq, s_wo, s_w1, s_w2 = range(8)
    small = [functools.partial(pltpu.make_async_copy, s, d, sem_w.at[i])
             for i, s, d in ((s_c, c_hbm, c_v), (s_x, x_hbm, x_v), (s_b1, b1_hbm, b1_v))]

    per_row = H * DH // LANE // PIECE
    w1_copies = flat(w1_hbm, w1_v, sem_w.at[s_w1])
    early = 84
    wide = 64

    def plain(src, dst, sem):
        return lambda i, o, k: pltpu.make_async_copy(src.at[pl.ds(i * PIECE + o, k)], dst.at[pl.ds(i * PIECE + o, k)], sem)

    parts = [(wmod_hbm.shape[0] // PIECE, plain(wmod_hbm, wmod_v, sem_w.at[s_wmod])),
             (early, plain(w1_hbm, w1_v, sem_w.at[s_w1])),
             (wo_hbm.shape[0] // PIECE, plain(wo_hbm, wo_v, sem_w.at[s_wo])),
             (wq_hbm.shape[0] // PIECE, plain(wq_hbm, wq_v, sem_w.at[s_wq]))]
    starts = [sum(n for n, _ in parts[:i]) for i in range(len(parts) + 1)]
    lines = starts[-1] // wide
    assert lines * wide == starts[-1]

    def columns(x, x0, shift=0, ramp=""):
        def piece(line, c):
            i = max(i for i, s0 in enumerate(starts) if s0 <= line * wide + x0)
            return functools.partial(parts[i][1], x + (line * wide + c - starts[i]))
        q0, q1 = [], []
        g = cfg["AG"]
        for c0, cut in ((0, (lines + 1) // 2 - shift), (2, lines // 2)):
            for out, mine in ((q0, range(cut)), (q1, range(cut, lines))):
                for i in range(0, len(mine), g):
                    out += [piece(line, c) for c in (c0, c0 + 1) for line in mine[i:i + g]]
        return _Stream(q0, q1, cfg["sa"], ramp)

    edges = sorted(set(s0 % wide for s0 in starts)) + [wide]
    if cfg["ramp"]:
        ramp = cfg["ramp"]
        st = columns(0, 0, (ramp.count("1") - ramp.count("0") + 2) // 4, ramp)
        for i in range(0, len(st.order), 4):
            st.more(4)
            fence()
        edges[0] = 4
    for cp in small:
        cp().start()
    for x0, x1 in zip(edges, edges[1:]):
        lax.fori_loop(x0 // 4, x1 // 4, lambda i, _, x0=x0: columns(i * 4, x0).rest(), None)
    mark("w")

    row = lax.broadcasted_iota(jnp.int32, (8, PAIR), 0)
    col = lax.broadcasted_iota(jnp.int32, (8, PAIR), 1)
    own = jnp.logical_or(jnp.logical_and(row == 0, col < DH), jnp.logical_and(row == 1, col >= DH))
    nd = D // LANE

    def query(p, st, step):
        if not compute:
            return
        parts = []
        for j in range(PAIR // LANE):
            parts.append(_dot(h1, column(wq_v, H * DH // LANE, p * (PAIR // LANE) + j, 0, D)))
            st.more(step)
        q_s[p] = jnp.where(own, jnp.concatenate(parts, axis=1), 0.0)

    def scores(p, h, st, step):
        slot = (p % 2) * 2 + h
        _wait_all(kv_v.at[slot], sem_kv.at[slot])
        if not compute:
            return
        q = q_s[p].astype(BF16)
        m = None if h == 0 else m_s[p]
        for c in range(half):
            s = _dot(q, kv_v[slot, c]) * DH ** -0.5
            s_s[p, h * half + c] = s
            m = s if m is None else jnp.maximum(m, s)
            st.more(step)
        m_s[p] = m

    def values(p, h, st, step, carry):
        slot = (p % 2) * 2 + h
        _wait_all(kv_v.at[slot], sem_kv.at[slot])
        if not compute:
            return None
        if h == 0:
            carry = (jnp.max(m_s[p], axis=-1, keepdims=True), jnp.zeros((8, LANE), F32), jnp.zeros((8, PAIR), F32))
        m, l, acc = carry
        for c in range(half):
            e = jnp.exp(s_s[p, h * half + c] - m)
            l += e
            acc += lax.dot_general(e.astype(BF16), kv_v[slot, c], (((1,), (1,)), ((), ())),
                                   preferred_element_type=F32)
            st.more(step)
        if h == 0:
            return m, l, acc
        return jnp.where(own, acc / jnp.sum(l, axis=-1, keepdims=True), 0.0)

    def project(p, o, st, step):
        if not compute:
            return 0.0
        o = o.astype(BF16)
        parts = []
        for j in range(nd):
            parts.append(_dot(o, column(wo_v, nd, j, p * PAIR, PAIR)))
            st.more(step)
        return jnp.concatenate(parts, axis=1)

    st = kv_stream(k_hbm, 0)
    st.more(look)
    for cp in small:
        cp().wait()
    _wait_all(wmod_v, sem_w.at[s_wmod])
    _wait_all(wq_v, sem_w.at[s_wq])
    _wait_all(wo_v, sem_w.at[s_wo])
    if compute:
        cf = c_v[...].astype(F32)
        silu_c = jnp.broadcast_to(cf * jax.nn.sigmoid(cf), (8, D)).astype(BF16)
        for j in range(6 * nd):
            mod_s[j // nd, :, j % nd * LANE:(j % nd + 1) * LANE] = _dot(silu_c, column(wmod_v, 6 * nd, j, 0, D))
            st.more(cfg["modstep"])
            if cfg["modfence"] and j % cfg["modfence"] == cfg["modfence"] - 1:
                fence()
        x0 = jnp.broadcast_to(x_v[...].astype(F32), (8, D))
        h1 = (_layernorm(x0) * (1.0 + mod_s[1]) + mod_s[0]).astype(BF16)
    query(0, st, 4)
    st.rest()
    sl = cfg.get("slook", 0)

    def loop(body):
        u = cfg.get("unroll", 1)

        def many(i, carry):
            for j in range(u):
                body(1 + i * u + j, carry)
            return carry

        lax.fori_loop(0, (NPAIR - 1) // u, many if u > 1 else lambda i, c: body(i + 1, c), 0)

    def k_body(p, carry):
        st = kv_stream(k_hbm, p)
        st.more(sl)
        scores(p - 1, 0, st, 5 if not sl else 2)
        st.upto(96)
        scores(p - 1, 1, st, 5)
        query(p, st, 5)
        st.rest()
        return carry

    mark("k0")
    loop(k_body)
    mark("k")

    st = kv_stream(v_hbm, 0)
    st.more(sl)
    scores(NPAIR - 1, 0, st, 5 if not sl else 2)
    st.upto(96)
    scores(NPAIR - 1, 1, st, 5)
    st.rest()
    if compute:
        o_s[...] = jnp.zeros(o_s.shape, F32)
        att_s[...] = jnp.zeros(att_s.shape, F32)

    def v_body(p, carry):
        st = kv_stream(v_hbm, p)
        if compute:
            att_s[...] += project(jnp.maximum(p - 2, 0), o_s[...], st, 3)
        st.upto(sl)
        c = values(p - 1, 0, st, 5 if not sl else 2, None)
        st.upto(96)
        o = values(p - 1, 1, st, 5, c)
        if compute:
            o_s[...] = o
        st.rest()
        return carry

    mark("v0")
    loop(v_body)
    mark("v")

    late = w1_copies[early:]
    q0, q1 = late[:len(late) // 2], late[len(late) // 2:]
    unit = cfg["unit"]
    per = unit // SUB * nd // PIECE
    nb = F // LANE
    groups = [runs for _, runs in cfg["w2_groups"]]
    assert sorted(u for runs in groups for a, b in runs for u in range(a, b)) == list(range(F // unit))
    for i, (queue, runs) in enumerate(cfg["w2_groups"]):
        pieces = flat(w2_hbm, w2_v, sem_w.at[s_w2 + i])
        lists = [pieces[a * per:b * per] for a, b in runs]
        (q0, q1)[queue].extend(l[k] for k in range(max(map(len, lists))) for l in lists if k < len(l))
    st = _Stream(q0, q1, cfg["st"])

    t0, t1, t2, t3 = cfg["tail"]
    st.upto(t0)
    fence()
    att = project(NPAIR - 2, o_s[...], st, 0) if compute else 0.0
    c = values(NPAIR - 1, 0, st, 0, None)
    fence()
    st.upto(t1)
    mark("pv")
    o = values(NPAIR - 1, 1, st, 0, c)
    fence()
    st.upto(t2)
    fence()
    att = att + project(NPAIR - 1, o, st, 0)
    if compute:
        att = jnp.broadcast_to(jnp.sum(att_s[...] + att, axis=0, keepdims=True), (8, D))
        x1 = x0 + mod_s[2] * att
        h2 = (_layernorm(x1) * (1.0 + mod_s[4]) + mod_s[3]).astype(BF16)
        b1 = b1_v[...].astype(F32)
    st.upto(t3)
    mark("h2")
    _wait_all(w1_v, sem_w.at[s_w1])
    if compute:
        u = [jnp.broadcast_to(b1[j:j + 1, :], (8, LANE)) + _dot(h2, column(w1_v, nb, j, 0, D)) for j in range(nb)]
        act = _mish(jnp.concatenate(u, axis=1)).astype(BF16)
        y = [jnp.zeros((8, LANE), F32)] * nd
    fence()
    st.rest()
    nv = cfg["vpu"]
    if compute:
        scale = {}
        for runs in groups[len(groups) - nv:]:
            for b0, b1_ in runs:
                for t in range(b0 * unit // LANE, -(-b1_ * unit // LANE)):
                    scale[t] = jnp.broadcast_to(act[0:1, t * LANE:(t + 1) * LANE].astype(F32), (LANE, LANE)).T
        part = [None] * nd
    for i, runs in enumerate(groups):
        _wait_all(w2_v.at[pl.ds(0, sum(b - a for a, b in runs) * per * PIECE)], sem_w.at[s_w2 + i])
        mark(f"w2_{i}")
        if not compute:
            continue
        for b0, b1_ in runs:
            if i < len(groups) - nv:
                a = act[:, b0 * unit:b1_ * unit]
                y = [y[j] + _dot(a, column(w2_v, nd, j, b0 * unit, (b1_ - b0) * unit)) for j in range(nd)]
                continue
            for r in range(b0 * unit, b1_ * unit, SUB):
                a = scale[r // LANE][r % LANE:r % LANE + SUB]
                for j in range(nd):
                    t = w2_v[r // SUB * nd + j].astype(F32) * a
                    part[j] = t if part[j] is None else part[j] + t
    if compute:
        out = x1 + mod_s[5] * jnp.concatenate(y, axis=1)
        if nv:
            out = out[0:1] + mod_s[5, 0:1] * jnp.sum(jnp.concatenate(part, axis=1), axis=0, keepdims=True)
        o_ref[...] = out[0:1].astype(o_ref.dtype)
    else:
        o_ref[...] = jnp.zeros(o_ref.shape, o_ref.dtype)


def _tiles(a):
    r, c = a.shape
    return a.reshape(r // SUB, SUB, c // LANE, LANE).transpose(0, 2, 1, 3)


def _flat(a):
    return _tiles(a).reshape(-1, SUB, LANE)


def make(**over):
    cfg = dict(DEFAULT)
    cfg.update(over)

    def fn(A_x, A_k_cache, A_v_cache, A_wq, A_wo, B_x, B_w1, B_b1, B_w2, c, w_mod):
        del B_x
        sk = A_k_cache.shape[2]
        window = min(4096, max(256, sk // 4))
        nc = window // LANE
        kt = _tiles(jnp.swapaxes(A_k_cache, 2, 3).reshape(H * DH, sk))
        vt = _tiles(jnp.swapaxes(A_v_cache, 2, 3).reshape(H * DH, sk))
        wmod, wo, w1, w2 = _flat(w_mod), _flat(A_wo), _flat(B_w1), _flat(B_w2)
        hbm = pl.BlockSpec(memory_space=pltpu.HBM)
        out = pl.pallas_call(
            functools.partial(_kernel, window=window, cfg=cfg),
            out_shape=jax.ShapeDtypeStruct((1, D), A_x.dtype),
            in_specs=[hbm] * 10,
            out_specs=pl.BlockSpec(memory_space=pltpu.VMEM),
            scratch_shapes=[
                pltpu.VMEM((1, D), BF16), pltpu.VMEM((1, D), BF16), pltpu.VMEM((F // LANE, LANE), BF16),
                pltpu.VMEM(wmod.shape, BF16),
                pltpu.VMEM(wo.shape, BF16),
                pltpu.VMEM(wo.shape, BF16), pltpu.VMEM(w1.shape, BF16), pltpu.VMEM(w2.shape, BF16),
                pltpu.VMEM((4, nc // 2, PAIR, LANE), BF16),
                pltpu.VMEM((NPAIR, 8, PAIR), F32),
                pltpu.VMEM((NPAIR, nc, 8, LANE), F32),
                pltpu.VMEM((NPAIR, 8, LANE), F32),
                pltpu.VMEM((8, PAIR), F32),
                pltpu.VMEM((8, D), F32),
                pltpu.VMEM((6, 8, D), F32),
                pltpu.SemaphoreType.DMA((7 + len(cfg["w2_groups"]),)),
                pltpu.SemaphoreType.DMA((4,)),
                pltpu.SemaphoreType.REGULAR,
            ],
            compiler_params=pltpu.CompilerParams(vmem_limit_bytes=64 * 2**20, disable_semaphore_checks=True,
                                                 disable_bounds_checks=not cfg["bounds"], flags=cfg.get("flags")),
            name="adaln_attn_mlp_decode",
        )(A_x.reshape(1, D), kt, vt, _flat(A_wq), wo, w1, B_b1.reshape(F // LANE, LANE), w2, c, wmod)
        return out.reshape(A_x.shape)
    return fn


pallas_adaLN_cond__sliding_block_cached__dense_activation_mish__decode_kernel = jax.jit(make())
```

```python
import functools

import jax
import jax.numpy as jnp
from jax import lax
import jax.experimental.pallas as pl
import jax.experimental.pallas.tpu as pltpu

D, H, DH, F = 640, 32, 192, 1536
PAIR = 2 * DH
NPAIR = H // 2
LANE = 128
SUB = 8
NSLOT = 4
PIECE = 8
F32, BF16 = jnp.float32, jnp.bfloat16

DEFAULT = dict(G=8, lag=2, AG=11, j2=20, look=64, compute=True, bounds=False,
               w2_groups=((0, ((0, 4), (8, 12))), (1, ((12, 16), (20, 22))), (0, ((4, 8),)), (1, ((22, 24), (16, 17))), (1, ((17, 19),)), (1, ((19, 20),))), fence=True, tail=(40, 96, 126, 150), pv_vpu=8, early=84, mix=0, j1=0,
               gather="stack", skv=(2, 2), sa=(2, 2), st=(1, 1), modstep=3, modfence=5, ramp="10111" * 5, w1_late=32, vpu=2, unit=64)


def _layernorm(x, eps=1e-5):
    m = jnp.mean(x, axis=-1, keepdims=True)
    d = x - m
    v = jnp.mean(d * d, axis=-1, keepdims=True)
    return d / jnp.sqrt(v + eps)


def _mish(u):
    softplus = jnp.log1p(jnp.exp(-jnp.abs(u))) + jnp.where(u > 0, u, 0.0)
    return u * jnp.tanh(softplus)


def _dot(a, b):
    return jnp.dot(a, b, preferred_element_type=F32)


def _dot_t(a, b):
    return lax.dot_general(a, b, (((1,), (1,)), ((), ())), preferred_element_type=F32)


def _walk(items, jump, k=1, group=10**9):
    out = []
    for o in range(0, jump, k):
        starts = list(range(o, len(items), jump))
        for g in range(0, len(starts), group):
            for c in range(min(k, jump - o)):
                out += [items[r + c] for r in starts[g:g + group] if r + c < len(items)]
    assert len(out) == len(items)
    return out


def _wait_all(buf, sem):
    pltpu.make_async_copy(buf, buf, sem).wait()


class _Stream:
    def __init__(self, q0, q1, split, ramp=""):
        lists, pos = (q0, q1), [0, 0]
        self.order = []
        self.split = split
        for queue in map(int, ramp):
            self.order.append((lists[queue][pos[queue]], queue))
            pos[queue] += 1
        while len(self.order) < len(q0) + len(q1):
            for queue in (0, 1):
                self.order += [(cp, queue) for cp in lists[queue][pos[queue]:pos[queue] + 2]]
                pos[queue] += 2
        self.pos = 0

    def more(self, n):
        for cp, queue in self.order[self.pos:self.pos + n]:
            k = PIECE // self.split[queue]
            for o in range(0, PIECE, k):
                cp(o, k).start(priority=queue)
        self.pos += n

    def upto(self, n):
        self.more(max(n - self.pos, 0))

    def rest(self):
        self.upto(len(self.order))


def _kernel(x_hbm, k_hbm, v_hbm, wq_hbm, wo_hbm, w1_hbm, b1_hbm, w2_hbm, c_hbm, wmod_hbm, o_ref,
            x_v, c_v, b1_v, wmod_v, wq_v, wo_v, w1_v, w2_v, kv_v, q_s, s_s, m_s, l_s, acc_s, att_s, mod_s,
            sem_w, sem_kv, sem_fence, *, window, cfg):
    nc = window // LANE
    c_first = k_hbm.shape[1] - nc
    half = nc // 2
    look = cfg["look"]
    compute = cfg["compute"]

    def mark(name):
        if cfg.get("marks"):
            with jax.named_scope("M_" + name):
                pl.delay(1)

    def fence():
        if cfg["fence"]:
            pl.semaphore_signal(sem_fence, 1)
            pl.semaphore_wait(sem_fence, 1)

    def flat(src, dst, sem):
        return [lambda o, k, i=i: pltpu.make_async_copy(src.at[pl.ds(i + o, k)], dst.at[pl.ds(i + o, k)], sem)
                for i in range(0, src.shape[0], PIECE)]

    def column(buf, ncol, j, row0, nrow):
        t0, n = row0 // SUB, nrow // SUB
        if cfg["gather"] == "stack":
            return jnp.stack([buf[(t0 + r) * ncol + j] for r in range(n)]).reshape(nrow, LANE)
        return buf[pl.ds(t0 * ncol + j, n, stride=ncol)].reshape(nrow, LANE)

    def kv_pieces(src, u):
        rows, g = PAIR // SUB, cfg["G"]
        row0, col0, slot = u % NPAIR * rows, c_first + u // NPAIR % 2 * half, u % NSLOT

        def piece(r, c):
            return lambda o, k: pltpu.make_async_copy(src.at[row0 + r, pl.ds(col0 + (c + o), k)],
                                                      kv_v.at[slot, pl.ds(c + o, k), pl.ds(r * SUB, SUB), :],
                                                      sem_kv.at[slot])
        return [[piece(r, c) for i in range(0, rows, 2 * g) for c in range(0, half, PIECE)
                 for r in range(i + parity, i + 2 * g, 2)] for parity in range(2)]

    lag = cfg["lag"]

    def kv_stream(src, u, before=None):
        q0, q1 = kv_pieces(src, u)
        late = [] if before is None or not lag else kv_pieces(before, u - 1)[1][-lag:]
        st = _Stream(q0, late + q1[:len(q1) - lag], cfg["skv"], "0" * (lag - len(late)))
        st.more(4)
        return st

    s_c, s_x, s_b1, s_wmod, s_wq, s_wo, s_w1, s_w2 = range(8)
    small = [functools.partial(pltpu.make_async_copy, s, d, sem_w.at[i])
             for i, s, d in ((s_c, c_hbm, c_v), (s_x, x_hbm, x_v), (s_b1, b1_hbm, b1_v))]

    per_row = H * DH // LANE // PIECE
    w1_copies = flat(w1_hbm, w1_v, sem_w.at[s_w1])
    early = cfg["early"]
    wide = 64

    def plain(src, dst, sem):
        return lambda i, o, k: pltpu.make_async_copy(src.at[pl.ds(i * PIECE + o, k)], dst.at[pl.ds(i * PIECE + o, k)], sem)

    parts = [(wmod_hbm.shape[0] // PIECE, plain(wmod_hbm, wmod_v, sem_w.at[s_wmod])),
             (early, plain(w1_hbm, w1_v, sem_w.at[s_w1])),
             (wo_hbm.shape[0] // PIECE, plain(wo_hbm, wo_v, sem_w.at[s_wo])),
             (wq_hbm.shape[0] // PIECE, plain(wq_hbm, wq_v, sem_w.at[s_wq]))]
    starts = [sum(n for n, _ in parts[:i]) for i in range(len(parts) + 1)]
    lines = starts[-1] // wide
    assert lines * wide == starts[-1]

    def columns(x, x0, shift=0, ramp=""):
        def piece(line, c):
            i = max(i for i, s0 in enumerate(starts) if s0 <= line * wide + x0)
            return functools.partial(parts[i][1], x + (line * wide + c - starts[i]))
        q0, q1 = [], []
        g = cfg["AG"]
        for c0, cut in ((0, (lines + 1) // 2 - shift), (2, lines // 2)):
            for out, mine in ((q0, range(cut)), (q1, range(cut, lines))):
                for i in range(0, len(mine), g):
                    out += [piece(line, c) for c in (c0, c0 + 1) for line in mine[i:i + g]]
        return _Stream(q0, q1, cfg["sa"], ramp)

    edges = sorted(set(s0 % wide for s0 in starts)) + [wide]
    if cfg["ramp"]:
        ramp = cfg["ramp"]
        st = columns(0, 0, (ramp.count("1") - ramp.count("0") + 2) // 4, ramp)
        for i in range(0, len(st.order), 4):
            st.more(4)
            fence()
        edges[0] = 4
    for cp in small:
        cp().start()
    for x0, x1 in zip(edges, edges[1:]):
        lax.fori_loop(x0 // 4, x1 // 4, lambda i, _, x0=x0: columns(i * 4, x0).rest(), None)
    mark("w")

    row = lax.broadcasted_iota(jnp.int32, (8, PAIR), 0)
    col = lax.broadcasted_iota(jnp.int32, (8, PAIR), 1)
    own = jnp.logical_or(jnp.logical_and(row == 0, col < DH), jnp.logical_and(row == 1, col >= DH))
    nd = D // LANE

    def query(p, st, step):
        if not compute:
            return
        parts = []
        for j in range(PAIR // LANE):
            parts.append(_dot(h1, column(wq_v, H * DH // LANE, p * (PAIR // LANE) + j, 0, D)))
            st.more(step)
        q_s[p] = jnp.where(own, jnp.concatenate(parts, axis=1), 0.0)

    def scores(u, st, step):
        p, h, slot = u % NPAIR, u // NPAIR, u % NSLOT
        _wait_all(kv_v.at[slot], sem_kv.at[slot])
        if not compute:
            return
        q = q_s[p].astype(BF16)
        m = m_s[p]
        for c in range(half):
            s = _dot(q, kv_v[slot, c]) * DH ** -0.5
            s_s[p, h * half + c] = s
            m = jnp.maximum(m, s)
            st.more(step)
        m_s[p] = m

    def values(u, h, st, step, on_vpu=0):
        p, slot = u % NPAIR, u % NSLOT
        _wait_all(kv_v.at[slot], sem_kv.at[slot])
        if not compute:
            return None
        m = jnp.max(m_s[p], axis=-1, keepdims=True)
        l, acc = (l_s[p], acc_s[p]) if h else (jnp.zeros((8, LANE), F32), jnp.zeros((8, PAIR), F32))
        weights = []
        for c in range(half):
            e = jnp.exp(s_s[p, h * half + c] - m)
            l += e
            if c < on_vpu:
                weights.append([jnp.broadcast_to(e[i:i + 1], (2 * SUB, LANE)) for i in range(2)])
            else:
                acc += _dot_t(e.astype(BF16), kv_v[slot, c])
            st.more(step)
        if on_vpu:
            rows = []
            for r in range(0, PAIR, 2 * SUB):
                terms = [kv_v[slot, c, r:r + 2 * SUB].astype(F32) * weights[c][r // DH] for c in range(on_vpu)]
                rows.append(functools.reduce(jnp.add, terms).astype(BF16))
            acc += _dot_t(jnp.ones((8, LANE), BF16), jnp.concatenate(rows, axis=0))
        if h:
            return jnp.where(own, acc / jnp.sum(l, axis=-1, keepdims=True), 0.0)
        l_s[p], acc_s[p] = l, acc

    def project(p, o, st, step):
        if not compute:
            return 0.0
        o = o.astype(BF16)
        parts = []
        for j in range(nd):
            parts.append(_dot(o, column(wo_v, nd, j, p * PAIR, PAIR)))
            st.more(step)
        return jnp.concatenate(parts, axis=1)

    st = kv_stream(k_hbm, 0)
    st.upto(look)
    for cp in small:
        cp().wait()
    _wait_all(wmod_v, sem_w.at[s_wmod])
    _wait_all(wq_v, sem_w.at[s_wq])
    _wait_all(wo_v, sem_w.at[s_wo])
    if compute:
        cf = c_v[...].astype(F32)
        silu_c = jnp.broadcast_to(cf * jax.nn.sigmoid(cf), (8, D)).astype(BF16)
    for i in range(6):
        if i == 2:
            st.rest()
            st = kv_stream(k_hbm, 1, k_hbm)
        if compute:
            for j in range(nd):
                mod_s[i, :, j * LANE:(j + 1) * LANE] = _dot(silu_c, column(wmod_v, 6 * nd, i * nd + j, 0, D))
                st.more(3)
        fence()
    if compute:
        x0 = jnp.broadcast_to(x_v[...].astype(F32), (8, D))
        h1 = (_layernorm(x0) * (1.0 + mod_s[1]) + mod_s[0]).astype(BF16)
        m_s[...] = jnp.full(m_s.shape, -jnp.inf, F32)
    query(0, st, 4)
    st.rest()

    def k_body(u, carry):
        st = kv_stream(k_hbm, u, k_hbm)
        scores(u - 2, st, 4)
        query((u - 1) % NPAIR, st, 5)
        st.rest()
        return carry

    mark("k0")
    lax.fori_loop(2, 2 * NPAIR, k_body, 0)
    mark("k")

    for u, before in ((2 * NPAIR, k_hbm), (2 * NPAIR + 1, v_hbm)):
        st = kv_stream(v_hbm, u, before)
        scores(u - 2, st, 5)
        st.rest()
    if compute:
        att_s[...] = jnp.zeros(att_s.shape, F32)

    def v_body(h, u, carry):
        st = kv_stream(v_hbm, u, v_hbm)
        o = values(u - 2, h, st, 5)
        if compute and h:
            att_s[...] += project((u - 2) % NPAIR, o, st, 2)
        st.rest()
        return carry

    mark("v0")
    lax.fori_loop(2 * NPAIR + 2, 3 * NPAIR + 2, functools.partial(v_body, 0), 0)
    lax.fori_loop(3 * NPAIR + 2, 4 * NPAIR, functools.partial(v_body, 1), 0)
    mark("v")

    late = w1_copies[early:]
    q0, q1 = late[:len(late) // 2], late[len(late) // 2:]
    if cfg["j1"]:
        q0, q1 = _walk(q0, cfg["j1"]), _walk(q1, cfg["j1"])
    n_late = len(q0)
    unit = cfg["unit"]
    per = unit // SUB * nd // PIECE
    nb = F // LANE
    groups = [runs for _, runs in cfg["w2_groups"]]
    assert sorted(u for runs in groups for a, b in runs for u in range(a, b)) == list(range(F // unit))
    for i, (queue, runs) in enumerate(cfg["w2_groups"]):
        pieces = flat(w2_hbm, w2_v, sem_w.at[s_w2 + i])
        lists = [pieces[a * per:b * per] for a, b in runs]
        (q0, q1)[queue].extend(l[k] for k in range(max(map(len, lists))) for l in lists if k < len(l))
    if cfg["mix"]:
        def mix(q):
            a, b = q[:n_late], q[n_late:n_late + cfg["mix"]]
            key = [((i + .5) / len(a), 0, i) for i in range(len(a))] + [((i + .5) / len(b), 1, i) for i in range(len(b))]
            return [(a, b)[k][i] for _, k, i in sorted(key)] + q[n_late + cfg["mix"]:]
        q0, q1 = mix(q0), mix(q1)
    if lag:
        q1 = kv_pieces(v_hbm, 4 * NPAIR - 1)[1][-lag:] + q1
    st = _Stream(q0, q1, cfg["st"])

    t0, t1, t2, t3 = cfg["tail"]
    st.more(4)
    fence()
    st.upto(t0)
    o0 = values(4 * NPAIR - 2, 1, st, 0, cfg["pv_vpu"])
    fence()
    st.upto(t1)
    mark("pv")
    o1 = values(4 * NPAIR - 1, 1, st, 0, cfg["pv_vpu"])
    fence()
    st.upto(t2)
    fence()
    att = project(NPAIR - 2, o0, st, 0) + project(NPAIR - 1, o1, st, 0)
    if compute:
        att = jnp.broadcast_to(jnp.sum(att_s[...] + att, axis=0, keepdims=True), (8, D))
        x1 = x0 + mod_s[2] * att
        h2 = (_layernorm(x1) * (1.0 + mod_s[4]) + mod_s[3]).astype(BF16)
        b1 = b1_v[...].astype(F32)
    st.upto(max(t3, 2 * (n_late + cfg["mix"]) + 2 * lag + 4))
    mark("h2")
    _wait_all(w1_v, sem_w.at[s_w1])
    if compute:
        u = [jnp.broadcast_to(b1[j:j + 1, :], (8, LANE)) + _dot(h2, column(w1_v, nb, j, 0, D)) for j in range(nb)]
        act = _mish(jnp.concatenate(u, axis=1)).astype(BF16)
        y = [jnp.zeros((8, LANE), F32)] * nd
    fence()
    st.rest()
    nv = cfg["vpu"]
    if compute:
        scale = {}
        for runs in groups[len(groups) - nv:]:
            for b0, b1_ in runs:
                for t in range(b0 * unit // LANE, -(-b1_ * unit // LANE)):
                    scale[t] = jnp.broadcast_to(act[0:1, t * LANE:(t + 1) * LANE].astype(F32), (LANE, LANE)).T
        part = [None] * nd
    for i, runs in enumerate(groups):
        _wait_all(w2_v.at[pl.ds(0, sum(b - a for a, b in runs) * per * PIECE)], sem_w.at[s_w2 + i])
        mark(f"w2_{i}")
        if not compute:
            continue
        for b0, b1_ in runs:
            if i < len(groups) - nv:
                a = act[:, b0 * unit:b1_ * unit]
                y = [y[j] + _dot(a, column(w2_v, nd, j, b0 * unit, (b1_ - b0) * unit)) for j in range(nd)]
                continue
            for r in range(b0 * unit, b1_ * unit, SUB):
                a = scale[r // LANE][r % LANE:r % LANE + SUB]
                for j in range(nd):
                    t = w2_v[r // SUB * nd + j].astype(F32) * a
                    part[j] = t if part[j] is None else part[j] + t
    if compute:
        out = x1 + mod_s[5] * jnp.concatenate(y, axis=1)
        if nv:
            out = out[0:1] + mod_s[5, 0:1] * jnp.sum(jnp.concatenate(part, axis=1), axis=0, keepdims=True)
        o_ref[...] = out[0:1].astype(o_ref.dtype)
    else:
        o_ref[...] = jnp.zeros(o_ref.shape, o_ref.dtype)


def _tiles(a):
    r, c = a.shape
    return a.reshape(r // SUB, SUB, c // LANE, LANE).transpose(0, 2, 1, 3)


def _flat(a):
    return _tiles(a).reshape(-1, SUB, LANE)


def make(**over):
    cfg = dict(DEFAULT)
    cfg.update(over)

    def fn(A_x, A_k_cache, A_v_cache, A_wq, A_wo, B_x, B_w1, B_b1, B_w2, c, w_mod):
        del B_x
        sk = A_k_cache.shape[2]
        window = min(4096, max(256, sk // 4))
        nc = window // LANE
        kt = _tiles(jnp.swapaxes(A_k_cache, 2, 3).reshape(H * DH, sk))
        vt = _tiles(jnp.swapaxes(A_v_cache, 2, 3).reshape(H * DH, sk))
        wmod, wo, w1, w2 = _flat(w_mod), _flat(A_wo), _flat(B_w1), _flat(B_w2)
        hbm = pl.BlockSpec(memory_space=pltpu.HBM)
        out = pl.pallas_call(
            functools.partial(_kernel, window=window, cfg=cfg),
            out_shape=jax.ShapeDtypeStruct((1, D), A_x.dtype),
            in_specs=[hbm] * 10,
            out_specs=pl.BlockSpec(memory_space=pltpu.VMEM),
            scratch_shapes=[
                pltpu.VMEM((1, D), BF16), pltpu.VMEM((1, D), BF16), pltpu.VMEM((F // LANE, LANE), BF16),
                pltpu.VMEM(wmod.shape, BF16),
                pltpu.VMEM(wo.shape, BF16),
                pltpu.VMEM(wo.shape, BF16), pltpu.VMEM(w1.shape, BF16), pltpu.VMEM(w2.shape, BF16),
                pltpu.VMEM((4, nc // 2, PAIR, LANE), BF16),
                pltpu.VMEM((NPAIR, 8, PAIR), F32),
                pltpu.VMEM((NPAIR, nc, 8, LANE), F32),
                pltpu.VMEM((NPAIR, 8, LANE), F32),
                pltpu.VMEM((NPAIR, 8, LANE), F32),
                pltpu.VMEM((NPAIR, 8, PAIR), F32),
                pltpu.VMEM((8, D), F32),
                pltpu.VMEM((6, 8, D), F32),
                pltpu.SemaphoreType.DMA((7 + len(cfg["w2_groups"]),)),
                pltpu.SemaphoreType.DMA((4,)),
                pltpu.SemaphoreType.REGULAR,
            ],
            compiler_params=pltpu.CompilerParams(vmem_limit_bytes=64 * 2**20, disable_semaphore_checks=True,
                                                 disable_bounds_checks=not cfg["bounds"], flags=cfg.get("flags")),
            name="adaln_attn_mlp_decode",
        )(A_x.reshape(1, D), kt, vt, _flat(A_wq), wo, w1, B_b1.reshape(F // LANE, LANE), w2, c, wmod)
        return out.reshape(A_x.shape)
    return fn


pallas_adaLN_cond__sliding_block_cached__dense_activation_mish__decode_kernel = jax.jit(make())
```

```python
import functools

import jax
import jax.numpy as jnp
from jax import lax
import jax.experimental.pallas as pl
import jax.experimental.pallas.tpu as pltpu

D = 640
H = 32
DH = 192
F = 1536
PAIR = 2 * DH
NPAIR = H // 2
SUB, LANE = 8, 128
F32 = jnp.float32
BF16 = jnp.bfloat16

PIECE = 8
NSLOT = 4
KV_GROUP = 16
KV_LAG = 2
LINE = 64
W1_EARLY = 84
RAMP = "10111" * 5
W2_UNIT = 64
W2_MXU = ((0, ((0, 4), (8, 12))), (1, ((12, 16), (20, 22))), (0, ((4, 8),)), (1, ((22, 24), (16, 17))))
W2_VPU = ((1, ((17, 19),)), (1, ((19, 20),)))
TAIL = (36, 96, 126, 150)


def _layernorm(x, eps=1e-5):
    m = jnp.mean(x, axis=-1, keepdims=True)
    d = x - m
    v = jnp.mean(d * d, axis=-1, keepdims=True)
    return d / jnp.sqrt(v + eps)


def _mish(u):
    softplus = jnp.log1p(jnp.exp(-jnp.abs(u))) + jnp.where(u > 0, u, 0.0)
    return u * jnp.tanh(softplus)


def _dot(a, b):
    return jnp.dot(a, b, preferred_element_type=F32)


def _dot_t(a, b):
    return lax.dot_general(a, b, (((1,), (1,)), ((), ())), preferred_element_type=F32)


def _column(buf, ncol, j, row0, nrow):
    t0 = row0 // SUB * ncol + j
    return jnp.stack([buf[t0 + r * ncol] for r in range(nrow // SUB)]).reshape(nrow, LANE)


def _piece(src, dst, sem, i):
    return lambda o, n: pltpu.make_async_copy(src.at[pl.ds(i * PIECE + o, n)], dst.at[pl.ds(i * PIECE + o, n)], sem)


def _wait_all(buf, sem):
    pltpu.make_async_copy(buf, buf, sem).wait()


class _Stream:
    def __init__(self, q0, q1, parts=2, opening=""):
        lists, pos = (q0, q1), [0, 0]
        self.order = []
        for queue in map(int, opening):
            self.order.append((lists[queue][pos[queue]], queue))
            pos[queue] += 1
        while len(self.order) < len(q0) + len(q1):
            for queue in (0, 1):
                self.order += [(piece, queue) for piece in lists[queue][pos[queue]:pos[queue] + 2]]
                pos[queue] += 2
        self.parts = parts
        self.pos = 0

    def more(self, n):
        for piece, queue in self.order[self.pos:self.pos + n]:
            size = PIECE // self.parts if queue else PIECE
            for o in range(0, PIECE, size):
                piece(o, size).start(priority=queue)
        self.pos += n

    def upto(self, n):
        self.more(max(n - self.pos, 0))

    def rest(self):
        self.upto(len(self.order))


def _kernel(x_hbm, k_hbm, v_hbm, wq_hbm, wo_hbm, w1_hbm, b1_hbm, w2_hbm, c_hbm, wmod_hbm, o_ref,
            x_v, c_v, b1_v, wmod_v, wq_v, wo_v, w1_v, w2_v, kv_v,
            mod_s, q_s, s_s, m_s, l_s, acc_s, att_s, out_s, sem_w, sem_kv, sem_fence):
    half = kv_v.shape[1]
    window_start = k_hbm.shape[1] - 2 * half
    nd, nf = D // LANE, F // LANE
    s_c, s_x, s_b1, s_wmod, s_wq, s_wo, s_w1, s_w2 = range(8)

    def fence():
        pl.semaphore_signal(sem_fence, 1)
        pl.semaphore_wait(sem_fence, 1)

    matrices = ((wmod_hbm, wmod_v, s_wmod), (w1_hbm, w1_v, s_w1), (wo_hbm, wo_v, s_wo), (wq_hbm, wq_v, s_wq))
    starts = [0]
    for src, _, s in matrices:
        starts.append(starts[-1] + (W1_EARLY if s == s_w1 else src.shape[0] // PIECE))
    lines = starts[-1] // LINE
    assert lines * LINE == starts[-1] and all(s % 4 == 0 for s in starts)

    def weights(x, like, opening=""):
        def piece(line, c):
            i = max(i for i, s in enumerate(starts) if s <= line * LINE + like)
            src, dst, s = matrices[i]
            return _piece(src, dst, sem_w.at[s], x + (line * LINE + c - starts[i]))

        q0, q1 = [], []
        skew = (opening.count("1") - opening.count("0") + 2) // 4
        for c0, cut in ((0, (lines + 1) // 2 - skew), (2, lines // 2)):
            q0 += [piece(line, c) for c in (c0, c0 + 1) for line in range(cut)]
            q1 += [piece(line, c) for c in (c0, c0 + 1) for line in range(cut, lines)]
        return _Stream(q0, q1, opening=opening)

    st = weights(0, 0, RAMP)
    while st.pos < len(st.order):
        st.more(4)
        fence()
    small = [pltpu.make_async_copy(src, dst, sem_w.at[s])
             for src, dst, s in ((c_hbm, c_v, s_c), (x_hbm, x_v, s_x), (b1_hbm, b1_v, s_b1))]
    for copy in small:
        copy.start()
    edges = [4] + sorted({s % LINE for s in starts} - {0}) + [LINE]
    for x0, x1 in zip(edges, edges[1:]):
        lax.fori_loop(x0 // 4, x1 // 4, lambda i, _, like=x0: weights(i * 4, like).rest(), None)

    def kv_pieces(src, u):
        rows = PAIR // SUB
        row0, col0, slot = u % NPAIR * rows, window_start + u // NPAIR % 2 * half, u % NSLOT

        def piece(r, c):
            return lambda o, n: pltpu.make_async_copy(
                src.at[row0 + r, pl.ds(col0 + (c + o), n)],
                kv_v.at[slot, pl.ds(c + o, n), pl.ds(r * SUB, SUB), :], sem_kv.at[slot])

        return [[piece(r, c) for i in range(0, rows, KV_GROUP) for c in range(0, half, PIECE)
                 for r in range(i + parity, i + KV_GROUP, 2)] for parity in range(2)]

    def kv_stream(src, u, before=None):
        q0, q1 = kv_pieces(src, u)
        left_over = [] if before is None else kv_pieces(before, u - 1)[1][-KV_LAG:]
        st = _Stream(q0, left_over + q1[:-KV_LAG], opening="0" * (KV_LAG - len(left_over)))
        st.more(4)
        return st

    row = lax.broadcasted_iota(jnp.int32, (8, PAIR), 0)
    col = lax.broadcasted_iota(jnp.int32, (8, PAIR), 1)
    own = jnp.logical_or(jnp.logical_and(row == 0, col < DH), jnp.logical_and(row == 1, col >= DH))

    def query(p, st):
        parts = []
        for j in range(PAIR // LANE):
            parts.append(_dot(h1, _column(wq_v, H * DH // LANE, p * (PAIR // LANE) + j, 0, D)))
            st.more(5)
        q_s[p] = jnp.where(own, jnp.concatenate(parts, axis=1), 0.0)

    def scores(u, st):
        p, h, slot = u % NPAIR, u // NPAIR, u % NSLOT
        _wait_all(kv_v.at[slot], sem_kv.at[slot])
        q = q_s[p].astype(BF16)
        m = m_s[p]
        for c in range(half):
            s = _dot(q, kv_v[slot, c]) * DH ** -0.5
            s_s[p, h * half + c] = s
            m = jnp.maximum(m, s)
            st.more(4)
        m_s[p] = m

    def values(u, h, st=None, on_vpu=0):
        p, slot = u % NPAIR, u % NSLOT
        _wait_all(kv_v.at[slot], sem_kv.at[slot])
        m = jnp.max(m_s[p], axis=-1, keepdims=True)
        l, acc = (l_s[p], acc_s[p]) if h else (jnp.zeros((8, LANE), F32), jnp.zeros((8, PAIR), F32))
        probs = []
        for c in range(half):
            e = jnp.exp(s_s[p, h * half + c] - m)
            l += e
            if c < on_vpu:
                probs.append([jnp.broadcast_to(e[i:i + 1], (2 * SUB, LANE)) for i in range(2)])
            else:
                acc += _dot_t(e.astype(BF16), kv_v[slot, c])
            if st is not None:
                st.more(5)
        if on_vpu:
            rows = [functools.reduce(jnp.add, [kv_v[slot, c, r:r + 2 * SUB].astype(F32) * probs[c][r // DH]
                                               for c in range(on_vpu)]).astype(BF16)
                    for r in range(0, PAIR, 2 * SUB)]
            acc += _dot_t(jnp.ones((8, LANE), BF16), jnp.concatenate(rows, axis=0))
        if h:
            return jnp.where(own, acc / jnp.sum(l, axis=-1, keepdims=True), 0.0).astype(BF16)
        l_s[p], acc_s[p] = l, acc

    def project(p, o):
        return jnp.concatenate([_dot(o, _column(wo_v, nd, j, p * PAIR, PAIR)) for j in range(nd)], axis=1)

    st = kv_stream(k_hbm, 0)
    st.upto(72)
    for copy in small:
        copy.wait()
    for _, buf, s in matrices:
        if s != s_w1:
            _wait_all(buf, sem_w.at[s])
    cf = c_v[...].astype(F32)
    silu_c = jnp.broadcast_to(cf * jax.nn.sigmoid(cf), (8, D)).astype(BF16)
    for i in range(6):
        if i == 2:
            st.rest()
            st = kv_stream(k_hbm, 1, k_hbm)
        for j in range(nd):
            mod_s[i, :, j * LANE:(j + 1) * LANE] = _dot(silu_c, _column(wmod_v, 6 * nd, i * nd + j, 0, D))
            st.more(3)
        fence()
    x0 = jnp.broadcast_to(x_v[...].astype(F32), (8, D))
    h1 = (_layernorm(x0) * (1.0 + mod_s[1]) + mod_s[0]).astype(BF16)
    m_s[...] = jnp.full(m_s.shape, -jnp.inf, F32)
    att_s[...] = jnp.zeros(att_s.shape, F32)
    query(0, st)
    st.rest()

    def k_body(u, _):
        st = kv_stream(k_hbm, u, k_hbm)
        scores(u - 2, st)
        query((u - 1) % NPAIR, st)
        st.rest()

    lax.fori_loop(2, 2 * NPAIR, k_body, None)
    for u, before in ((2 * NPAIR, k_hbm), (2 * NPAIR + 1, v_hbm)):
        st = kv_stream(v_hbm, u, before)
        scores(u - 2, st)
        st.rest()

    def v_body(h, u, _):
        st = kv_stream(v_hbm, u, v_hbm)
        o = values(u - 2, h, st)
        if h:
            att_s[...] += project((u - 2) % NPAIR, o)
        st.rest()

    last = 4 * NPAIR - 1
    lax.fori_loop(2 * NPAIR + 2, 3 * NPAIR + 2, functools.partial(v_body, 0), None)
    lax.fori_loop(3 * NPAIR + 2, last + 1, functools.partial(v_body, 1), None)

    late = [_piece(w1_hbm, w1_v, sem_w.at[s_w1], i) for i in range(W1_EARLY, w1_hbm.shape[0] // PIECE)]
    queues = late[:len(late) // 2], kv_pieces(v_hbm, last)[1][-KV_LAG:] + late[len(late) // 2:]
    per = W2_UNIT // SUB * nd // PIECE
    for i, (queue, ranges) in enumerate(W2_MXU + W2_VPU):
        order = sorted((k - a * per, k) for a, b in ranges for k in range(a * per, b * per))
        queues[queue].extend(_piece(w2_hbm, w2_v, sem_w.at[s_w2 + i], k) for _, k in order)
    st = _Stream(*queues, parts=1)
    st.more(4)
    fence()
    st.upto(TAIL[0])
    o0 = values(last - 1, 1, on_vpu=half // 2)
    fence()
    st.upto(TAIL[1])
    o1 = values(last, 1, on_vpu=half // 2)
    fence()
    st.upto(TAIL[2])
    fence()

    att = att_s[...] + project(NPAIR - 2, o0) + project(NPAIR - 1, o1)
    x1 = x0 + mod_s[2] * jnp.broadcast_to(jnp.sum(att, axis=0, keepdims=True), (8, D))
    h2 = (_layernorm(x1) * (1.0 + mod_s[4]) + mod_s[3]).astype(BF16)
    b1 = b1_v[...].astype(F32)
    st.upto(TAIL[3])
    _wait_all(w1_v, sem_w.at[s_w1])
    up = [jnp.broadcast_to(b1[j:j + 1, :], (8, LANE)) + _dot(h2, _column(w1_v, nf, j, 0, D)) for j in range(nf)]
    act = _mish(jnp.concatenate(up, axis=1)).astype(BF16)
    fence()
    st.rest()

    tiles = sorted({r // LANE for _, ranges in W2_VPU for a, b in ranges for r in range(a * W2_UNIT, b * W2_UNIT, SUB)})
    scale = {t: jnp.broadcast_to(act[0:1, t * LANE:(t + 1) * LANE].astype(F32), (LANE, LANE)).T for t in tiles}

    def arrived(i, ranges):
        for a, b in ranges:
            _wait_all(w2_v.at[pl.ds(a * per * PIECE, (b - a) * per * PIECE)], sem_w.at[s_w2 + i])
        return [(a * W2_UNIT, b * W2_UNIT) for a, b in ranges]

    y = jnp.zeros((8, D), F32)
    for i, (_, ranges) in enumerate(W2_MXU):
        for r0, r1 in arrived(i, ranges):
            y += jnp.concatenate([_dot(act[:, r0:r1], _column(w2_v, nd, j, r0, r1 - r0)) for j in range(nd)], axis=1)
    out_s[...] = (x1 + mod_s[5] * y)[0:1]
    terms = [[] for _ in range(nd)]
    for i, (_, ranges) in enumerate(W2_VPU):
        for r0, r1 in arrived(len(W2_MXU) + i, ranges):
            for r in range(r0, r1, SUB):
                a = scale[r // LANE][r % LANE:r % LANE + SUB]
                for j in range(nd):
                    term = w2_v[r // SUB * nd + j].astype(F32) * a
                    terms[j] = [terms[j][0] + term] if terms[j] else [term]
    y = jnp.sum(jnp.concatenate([t[0] for t in terms], axis=1), axis=0, keepdims=True)
    o_ref[...] = (out_s[...] + mod_s[5, 0:1] * y).astype(o_ref.dtype)


def _tiles(a):
    r, c = a.shape
    return a.reshape(r // SUB, SUB, c // LANE, LANE).transpose(0, 2, 1, 3)


@jax.jit
def pallas_adaLN_cond__sliding_block_cached__dense_activation_mish__decode_kernel(
    A_x: jax.Array,
    A_k_cache: jax.Array,
    A_v_cache: jax.Array,
    A_wq: jax.Array,
    A_wo: jax.Array,
    B_x: jax.Array,
    B_w1: jax.Array,
    B_b1: jax.Array,
    B_w2: jax.Array,
    c: jax.Array,
    w_mod: jax.Array,
):
    del B_x
    sk = A_k_cache.shape[2]
    half = min(4096, max(256, sk // 4)) // LANE // 2
    kt, vt = (_tiles(jnp.swapaxes(a, 2, 3).reshape(H * DH, sk)) for a in (A_k_cache, A_v_cache))
    wmod, wq, wo, w1, w2 = (_tiles(a).reshape(-1, SUB, LANE) for a in (w_mod, A_wq, A_wo, B_w1, B_w2))
    out = pl.pallas_call(
        _kernel,
        out_shape=jax.ShapeDtypeStruct((1, D), A_x.dtype),
        in_specs=[pl.BlockSpec(memory_space=pltpu.HBM)] * 10,
        out_specs=pl.BlockSpec(memory_space=pltpu.VMEM),
        scratch_shapes=[
            pltpu.VMEM((1, D), BF16),
            pltpu.VMEM((1, D), BF16),
            pltpu.VMEM((F // LANE, LANE), BF16),
            *(pltpu.VMEM(a.shape, BF16) for a in (wmod, wq, wo, w1, w2)),
            pltpu.VMEM((NSLOT, half, PAIR, LANE), BF16),
            pltpu.VMEM((6, 8, D), F32),
            pltpu.VMEM((NPAIR, 8, PAIR), F32),
            pltpu.VMEM((NPAIR, 2 * half, 8, LANE), F32),
            pltpu.VMEM((NPAIR, 8, LANE), F32),
            pltpu.VMEM((NPAIR, 8, LANE), F32),
            pltpu.VMEM((NPAIR, 8, PAIR), F32),
            pltpu.VMEM((8, D), F32),
            pltpu.VMEM((1, D), F32),
            pltpu.SemaphoreType.DMA((7 + len(W2_MXU + W2_VPU),)),
            pltpu.SemaphoreType.DMA((NSLOT,)),
            pltpu.SemaphoreType.REGULAR,
        ],
        compiler_params=pltpu.CompilerParams(
            vmem_limit_bytes=64 * 2**20,
            disable_semaphore_checks=True,
        ),
        name="adaln_attn_mlp_decode",
    )(A_x.reshape(1, D), kt, vt, wq, wo, w1, B_b1.reshape(F // LANE, LANE), w2, c, wmod)
    return out.reshape(A_x.shape)
```

```python
import functools

import jax
import jax.numpy as jnp
from jax import lax
import jax.experimental.pallas as pl
import jax.experimental.pallas.tpu as pltpu

D = 640
H = 32
DH = 192
F = 1536
PAIR = 2 * DH
NPAIR = H // 2
SUB, LANE = 8, 128
F32 = jnp.float32
BF16 = jnp.bfloat16

PIECE = 8
NSLOT = 4
KV_GROUP = 16
KV_LAG = 2
LINE = 64
W1_EARLY = 84
RAMP = "10111" * 5
W2_MXU = ((0, ((0, 20), (40, 60))), (1, ((60, 80), (100, 110))), (0, ((20, 40),)), (1, ((110, 120), (80, 85))))
W2_VPU = ((1, ((85, 92),)), (1, ((92, 97),)), (1, ((97, 99),)), (1, ((99, 100),)))
TAIL = (36, 96, 126, 150)


def _layernorm(x, eps=1e-5):
    m = jnp.mean(x, axis=-1, keepdims=True)
    d = x - m
    v = jnp.mean(d * d, axis=-1, keepdims=True)
    return d / jnp.sqrt(v + eps)


def _mish(u):
    softplus = jnp.log1p(jnp.exp(-jnp.abs(u))) + jnp.where(u > 0, u, 0.0)
    return u * jnp.tanh(softplus)


def _dot(a, b):
    return jnp.dot(a, b, preferred_element_type=F32)


def _dot_t(a, b):
    return lax.dot_general(a, b, (((1,), (1,)), ((), ())), preferred_element_type=F32)


def _column(buf, ncol, j, row0, nrow):
    t0 = row0 // SUB * ncol + j
    return jnp.stack([buf[t0 + r * ncol] for r in range(nrow // SUB)]).reshape(nrow, LANE)


def _piece(src, dst, sem, i):
    return lambda o, n: pltpu.make_async_copy(src.at[pl.ds(i * PIECE + o, n)], dst.at[pl.ds(i * PIECE + o, n)], sem)


def _wait_all(buf, sem):
    pltpu.make_async_copy(buf, buf, sem).wait()


class _Stream:
    def __init__(self, q0, q1, parts=2, opening=""):
        lists, pos = (q0, q1), [0, 0]
        self.order = []
        for queue in map(int, opening):
            self.order.append((lists[queue][pos[queue]], queue))
            pos[queue] += 1
        while len(self.order) < len(q0) + len(q1):
            for queue in (0, 1):
                self.order += [(piece, queue) for piece in lists[queue][pos[queue]:pos[queue] + 2]]
                pos[queue] += 2
        self.parts = parts
        self.pos = 0

    def more(self, n):
        for piece, queue in self.order[self.pos:self.pos + n]:
            size = PIECE // self.parts if queue else PIECE
            for o in range(0, PIECE, size):
                piece(o, size).start(priority=queue)
        self.pos += n

    def upto(self, n):
        self.more(max(n - self.pos, 0))

    def rest(self):
        self.upto(len(self.order))


def _kernel(x_hbm, k_hbm, v_hbm, wq_hbm, wo_hbm, w1_hbm, b1_hbm, w2_hbm, c_hbm, wmod_hbm, o_ref,
            x_v, c_v, b1_v, wmod_v, wq_v, wo_v, w1_v, w2_v, kv_v,
            mod_s, q_s, s_s, m_s, l_s, acc_s, att_s, sem_w, sem_kv, sem_fence):
    half = kv_v.shape[1]
    window_start = k_hbm.shape[1] - 2 * half
    nd, nf = D // LANE, F // LANE
    s_c, s_x, s_b1, s_wmod, s_wq, s_wo, s_w1, s_w2 = range(8)

    def fence():
        pl.semaphore_signal(sem_fence, 1)
        pl.semaphore_wait(sem_fence, 1)

    matrices = ((wmod_hbm, wmod_v, s_wmod), (w1_hbm, w1_v, s_w1), (wo_hbm, wo_v, s_wo), (wq_hbm, wq_v, s_wq))
    starts = [0]
    for src, _, s in matrices:
        starts.append(starts[-1] + (W1_EARLY if s == s_w1 else src.shape[0] // PIECE))
    lines = starts[-1] // LINE
    assert lines * LINE == starts[-1] and all(s % 4 == 0 for s in starts)

    def weights(x, like, opening=""):
        def piece(line, c):
            i = max(i for i, s in enumerate(starts) if s <= line * LINE + like)
            src, dst, s = matrices[i]
            return _piece(src, dst, sem_w.at[s], x + (line * LINE + c - starts[i]))

        q0, q1 = [], []
        skew = (opening.count("1") - opening.count("0") + 2) // 4
        for c0, cut in ((0, (lines + 1) // 2 - skew), (2, lines // 2)):
            q0 += [piece(line, c) for c in (c0, c0 + 1) for line in range(cut)]
            q1 += [piece(line, c) for c in (c0, c0 + 1) for line in range(cut, lines)]
        return _Stream(q0, q1, opening=opening)

    st = weights(0, 0, RAMP)
    while st.pos < len(st.order):
        st.more(4)
        fence()
    small = [pltpu.make_async_copy(src, dst, sem_w.at[s])
             for src, dst, s in ((c_hbm, c_v, s_c), (x_hbm, x_v, s_x), (b1_hbm, b1_v, s_b1))]
    for copy in small:
        copy.start()
    edges = [4] + sorted({s % LINE for s in starts} - {0}) + [LINE]
    for x0, x1 in zip(edges, edges[1:]):
        lax.fori_loop(x0 // 4, x1 // 4, lambda i, _, like=x0: weights(i * 4, like).rest(), None)

    def kv_pieces(src, u):
        rows = PAIR // SUB
        row0, col0, slot = u % NPAIR * rows, window_start + u // NPAIR % 2 * half, u % NSLOT

        def piece(r, c):
            return lambda o, n: pltpu.make_async_copy(
                src.at[row0 + r, pl.ds(col0 + (c + o), n)],
                kv_v.at[slot, pl.ds(c + o, n), pl.ds(r * SUB, SUB), :], sem_kv.at[slot])

        return [[piece(r, c) for i in range(0, rows, KV_GROUP) for c in range(0, half, PIECE)
                 for r in range(i + parity, i + KV_GROUP, 2)] for parity in range(2)]

    def kv_stream(src, u, before=None):
        q0, q1 = kv_pieces(src, u)
        left_over = [] if before is None else kv_pieces(before, u - 1)[1][-KV_LAG:]
        st = _Stream(q0, left_over + q1[:-KV_LAG], opening="0" * (KV_LAG - len(left_over)))
        st.more(4)
        return st

    row = lax.broadcasted_iota(jnp.int32, (8, PAIR), 0)
    col = lax.broadcasted_iota(jnp.int32, (8, PAIR), 1)
    own = jnp.logical_or(jnp.logical_and(row == 0, col < DH), jnp.logical_and(row == 1, col >= DH))

    def query(p, st):
        parts = []
        for j in range(PAIR // LANE):
            parts.append(_dot(h1, _column(wq_v, H * DH // LANE, p * (PAIR // LANE) + j, 0, D)))
            st.more(5)
        q_s[p] = jnp.where(own, jnp.concatenate(parts, axis=1), 0.0)

    def scores(u, st):
        p, h, slot = u % NPAIR, u // NPAIR, u % NSLOT
        _wait_all(kv_v.at[slot], sem_kv.at[slot])
        q = q_s[p].astype(BF16)
        m = m_s[p]
        for c in range(half):
            s = _dot(q, kv_v[slot, c]) * DH ** -0.5
            s_s[p, h * half + c] = s
            m = jnp.maximum(m, s)
            st.more(4)
        m_s[p] = m

    def values(u, h, st=None, on_vpu=0):
        p, slot = u % NPAIR, u % NSLOT
        _wait_all(kv_v.at[slot], sem_kv.at[slot])
        m = jnp.max(m_s[p], axis=-1, keepdims=True)
        l, acc = (l_s[p], acc_s[p]) if h else (jnp.zeros((8, LANE), F32), jnp.zeros((8, PAIR), F32))
        probs = []
        for c in range(half):
            e = jnp.exp(s_s[p, h * half + c] - m)
            l += e
            if c < on_vpu:
                probs.append([jnp.broadcast_to(e[i:i + 1], (2 * SUB, LANE)) for i in range(2)])
            else:
                acc += _dot_t(e.astype(BF16), kv_v[slot, c])
            if st is not None:
                st.more(5)
        if on_vpu:
            rows = [functools.reduce(jnp.add, [kv_v[slot, c, r:r + 2 * SUB].astype(F32) * probs[c][r // DH]
                                               for c in range(on_vpu)]).astype(BF16)
                    for r in range(0, PAIR, 2 * SUB)]
            acc += _dot_t(jnp.ones((8, LANE), BF16), jnp.concatenate(rows, axis=0))
        if h:
            return jnp.where(own, acc / jnp.sum(l, axis=-1, keepdims=True), 0.0).astype(BF16)
        l_s[p], acc_s[p] = l, acc

    def project(p, o):
        return jnp.concatenate([_dot(o, _column(wo_v, nd, j, p * PAIR, PAIR)) for j in range(nd)], axis=1)

    st = kv_stream(k_hbm, 0)
    st.upto(72)
    for copy in small:
        copy.wait()
    for _, buf, s in matrices:
        if s != s_w1:
            _wait_all(buf, sem_w.at[s])
    cf = c_v[...].astype(F32)
    silu_c = jnp.broadcast_to(cf * jax.nn.sigmoid(cf), (8, D)).astype(BF16)
    for i in range(6):
        if i == 2:
            st.rest()
            st = kv_stream(k_hbm, 1, k_hbm)
        for j in range(nd):
            mod_s[i, :, j * LANE:(j + 1) * LANE] = _dot(silu_c, _column(wmod_v, 6 * nd, i * nd + j, 0, D))
            st.more(3)
        fence()
    x0 = jnp.broadcast_to(x_v[...].astype(F32), (8, D))
    h1 = (_layernorm(x0) * (1.0 + mod_s[1]) + mod_s[0]).astype(BF16)
    m_s[...] = jnp.full(m_s.shape, -jnp.inf, F32)
    att_s[...] = jnp.zeros(att_s.shape, F32)
    query(0, st)
    st.rest()

    def k_body(u, _):
        st = kv_stream(k_hbm, u, k_hbm)
        scores(u - 2, st)
        query((u - 1) % NPAIR, st)
        st.rest()

    lax.fori_loop(2, 2 * NPAIR, k_body, None)
    for u, before in ((2 * NPAIR, k_hbm), (2 * NPAIR + 1, v_hbm)):
        st = kv_stream(v_hbm, u, before)
        scores(u - 2, st)
        st.rest()

    def v_body(h, u, _):
        st = kv_stream(v_hbm, u, v_hbm)
        o = values(u - 2, h, st)
        if h:
            att_s[...] += project((u - 2) % NPAIR, o)
        st.rest()

    last = 4 * NPAIR - 1
    lax.fori_loop(2 * NPAIR + 2, 3 * NPAIR + 2, functools.partial(v_body, 0), None)
    lax.fori_loop(3 * NPAIR + 2, last + 1, functools.partial(v_body, 1), None)

    late = [_piece(w1_hbm, w1_v, sem_w.at[s_w1], i) for i in range(W1_EARLY, w1_hbm.shape[0] // PIECE)]
    queues = late[:len(late) // 2], kv_pieces(v_hbm, last)[1][-KV_LAG:] + late[len(late) // 2:]
    for i, (queue, ranges) in enumerate(W2_MXU + W2_VPU):
        order = sorted((k - a, k) for a, b in ranges for k in range(a, b))
        queues[queue].extend(_piece(w2_hbm, w2_v, sem_w.at[s_w2 + i], k) for _, k in order)
    st = _Stream(*queues, parts=1)
    st.more(4)
    fence()
    st.upto(TAIL[0])
    o0 = values(last - 1, 1, on_vpu=half // 2)
    fence()
    st.upto(TAIL[1])
    o1 = values(last, 1, on_vpu=half // 2)
    fence()
    st.upto(TAIL[2])
    fence()

    att = att_s[...] + project(NPAIR - 2, o0) + project(NPAIR - 1, o1)
    x1 = x0 + mod_s[2] * jnp.broadcast_to(jnp.sum(att, axis=0, keepdims=True), (8, D))
    h2 = (_layernorm(x1) * (1.0 + mod_s[4]) + mod_s[3]).astype(BF16)
    b1 = b1_v[...].astype(F32)
    st.upto(TAIL[3])
    _wait_all(w1_v, sem_w.at[s_w1])
    up = [jnp.broadcast_to(b1[j:j + 1, :], (8, LANE)) + _dot(h2, _column(w1_v, nf, j, 0, D)) for j in range(nf)]
    act = _mish(jnp.concatenate(up, axis=1)).astype(BF16)
    fence()
    st.rest()

    tiles = [t for _, ranges in W2_VPU for a, b in ranges for t in range(a * PIECE, b * PIECE)]
    act_t = {j: jnp.broadcast_to(act[0:1, j * LANE:(j + 1) * LANE].astype(F32), (LANE, LANE)).T
             for j in sorted({t // nd * SUB // LANE for t in tiles})}
    factor = {}
    for t in tiles:
        r, j = t // nd * SUB, t % nd
        factor[t] = act_t[r // LANE][r % LANE:r % LANE + SUB] * mod_s[5, :, j * LANE:(j + 1) * LANE]

    def arrived(i, ranges):
        for a, b in ranges:
            _wait_all(w2_v.at[pl.ds(a * PIECE, (b - a) * PIECE)], sem_w.at[s_w2 + i])
        return [(a * PIECE, b * PIECE) for a, b in ranges]

    y = jnp.zeros((8, D), F32)
    for i, (_, ranges) in enumerate(W2_MXU):
        for t0, t1 in arrived(i, ranges):
            r0, r1 = t0 // nd * SUB, t1 // nd * SUB
            y += jnp.concatenate([_dot(act[:, r0:r1], _column(w2_v, nd, j, r0, r1 - r0)) for j in range(nd)], axis=1)
    out = jnp.where(lax.broadcasted_iota(jnp.int32, (8, D), 0) == 0, x1 + mod_s[5] * y, 0.0)
    out = [out[:, j * LANE:(j + 1) * LANE] for j in range(nd)]
    for i, (_, ranges) in enumerate(W2_VPU):
        for t0, t1 in arrived(len(W2_MXU) + i, ranges):
            for t in range(t0, t1):
                out[t % nd] += w2_v[t].astype(F32) * factor[t]
    o_ref[...] = jnp.sum(jnp.concatenate(out, axis=1), axis=0, keepdims=True).astype(o_ref.dtype)


def _tiles(a):
    r, c = a.shape
    return a.reshape(r // SUB, SUB, c // LANE, LANE).transpose(0, 2, 1, 3)


@jax.jit
def pallas_adaLN_cond__sliding_block_cached__dense_activation_mish__decode_kernel(
    A_x: jax.Array,
    A_k_cache: jax.Array,
    A_v_cache: jax.Array,
    A_wq: jax.Array,
    A_wo: jax.Array,
    B_x: jax.Array,
    B_w1: jax.Array,
    B_b1: jax.Array,
    B_w2: jax.Array,
    c: jax.Array,
    w_mod: jax.Array,
):
    del B_x
    sk = A_k_cache.shape[2]
    half = min(4096, max(256, sk // 4)) // LANE // 2
    kt, vt = (_tiles(jnp.swapaxes(a, 2, 3).reshape(H * DH, sk)) for a in (A_k_cache, A_v_cache))
    wmod, wq, wo, w1, w2 = (_tiles(a).reshape(-1, SUB, LANE) for a in (w_mod, A_wq, A_wo, B_w1, B_w2))
    out = pl.pallas_call(
        _kernel,
        out_shape=jax.ShapeDtypeStruct((1, D), A_x.dtype),
        in_specs=[pl.BlockSpec(memory_space=pltpu.HBM)] * 10,
        out_specs=pl.BlockSpec(memory_space=pltpu.VMEM),
        scratch_shapes=[
            pltpu.VMEM((1, D), BF16),
            pltpu.VMEM((1, D), BF16),
            pltpu.VMEM((F // LANE, LANE), BF16),
            *(pltpu.VMEM(a.shape, BF16) for a in (wmod, wq, wo, w1, w2)),
            pltpu.VMEM((NSLOT, half, PAIR, LANE), BF16),
            pltpu.VMEM((6, 8, D), F32),
            pltpu.VMEM((NPAIR, 8, PAIR), F32),
            pltpu.VMEM((NPAIR, 2 * half, 8, LANE), F32),
            pltpu.VMEM((NPAIR, 8, LANE), F32),
            pltpu.VMEM((NPAIR, 8, LANE), F32),
            pltpu.VMEM((NPAIR, 8, PAIR), F32),
            pltpu.VMEM((8, D), F32),
            pltpu.SemaphoreType.DMA((7 + len(W2_MXU + W2_VPU),)),
            pltpu.SemaphoreType.DMA((NSLOT,)),
            pltpu.SemaphoreType.REGULAR,
        ],
        compiler_params=pltpu.CompilerParams(
            vmem_limit_bytes=64 * 2**20,
            disable_semaphore_checks=True,
        ),
        name="adaln_attn_mlp_decode",
    )(A_x.reshape(1, D), kt, vt, wq, wo, w1, B_b1.reshape(F // LANE, LANE), w2, c, wmod)
    return out.reshape(A_x.shape)
```

```python
import functools

import jax
import jax.numpy as jnp
from jax import lax
import jax.experimental.pallas as pl
import jax.experimental.pallas.tpu as pltpu

D = 640
H = 32
DH = 192
F = 1536
PAIR = 2 * DH
NPAIR = H // 2
SUB, LANE = 8, 128
F32 = jnp.float32
BF16 = jnp.bfloat16

PIECE = 8
NSLOT = 4
KV_LAG = 4
LINE = 64
W1_EARLY = 84
RAMP = "10111" * 5
W2_MXU = ((0, ((0, 20), (40, 60))), (1, ((60, 80), (100, 110))), (0, ((20, 40),)), (1, ((110, 120), (80, 85))))
W2_VPU = ((1, ((85, 92),)), (1, ((92, 97),)), (1, ((97, 99),)), (1, ((99, 100),)))
TAIL = (40, 80, 120, 150)


def _layernorm(x, eps=1e-5):
    m = jnp.mean(x, axis=-1, keepdims=True)
    d = x - m
    v = jnp.mean(d * d, axis=-1, keepdims=True)
    return d / jnp.sqrt(v + eps)


def _mish(u):
    softplus = jnp.log1p(jnp.exp(-jnp.abs(u))) + jnp.where(u > 0, u, 0.0)
    return u * jnp.tanh(softplus)


def _dot(a, b):
    return jnp.dot(a, b, preferred_element_type=F32)


def _dot_t(a, b):
    return lax.dot_general(a, b, (((1,), (1,)), ((), ())), preferred_element_type=F32)


def _column(buf, ncol, j, row0, nrow):
    t0 = row0 // SUB * ncol + j
    return jnp.stack([buf[t0 + r * ncol] for r in range(nrow // SUB)]).reshape(nrow, LANE)


def _piece(src, dst, sem, i):
    return lambda o, n: pltpu.make_async_copy(src.at[pl.ds(i * PIECE + o, n)], dst.at[pl.ds(i * PIECE + o, n)], sem)


def _wait_all(buf, sem):
    pltpu.make_async_copy(buf, buf, sem).wait()


class _Stream:
    def __init__(self, q0, q1, parts=2, opening=""):
        lists, pos = (q0, q1), [0, 0]
        self.order = []
        for queue in map(int, opening):
            self.order.append((lists[queue][pos[queue]], queue))
            pos[queue] += 1
        while len(self.order) < len(q0) + len(q1):
            for queue in (0, 1):
                self.order += [(piece, queue) for piece in lists[queue][pos[queue]:pos[queue] + 2]]
                pos[queue] += 2
        self.parts = parts
        self.pos = 0

    def more(self, n):
        for piece, queue in self.order[self.pos:self.pos + n]:
            size = PIECE // self.parts if queue else PIECE
            for o in range(0, PIECE, size):
                piece(o, size).start(priority=queue)
        self.pos += n

    def upto(self, n):
        self.more(max(n - self.pos, 0))

    def rest(self):
        self.upto(len(self.order))


def _kernel(x_hbm, k_hbm, v_hbm, wq_hbm, wo_hbm, w1_hbm, b1_hbm, w2_hbm, c_hbm, wmod_hbm, o_ref,
            x_v, c_v, b1_v, wmod_v, wq_v, wo_v, w1_v, w2_v, kv_v,
            mod_s, q_s, s_s, m_s, l_s, acc_s, att_s, sem_w, sem_kv, sem_fence):
    passes = s_s.shape[1] // PIECE
    window_start = k_hbm.shape[1] - passes * PIECE
    nu = passes * NPAIR
    nd, nf = D // LANE, F // LANE
    s_c, s_x, s_b1, s_wmod, s_wq, s_wo, s_w1, s_w2 = range(8)

    def fence():
        pl.semaphore_signal(sem_fence, 1)
        pl.semaphore_wait(sem_fence, 1)

    matrices = ((wmod_hbm, wmod_v, s_wmod), (w1_hbm, w1_v, s_w1), (wo_hbm, wo_v, s_wo), (wq_hbm, wq_v, s_wq))
    starts = [0]
    for src, _, s in matrices:
        starts.append(starts[-1] + (W1_EARLY if s == s_w1 else src.shape[0] // PIECE))
    lines = starts[-1] // LINE
    assert lines * LINE == starts[-1] and all(s % 4 == 0 for s in starts)

    def weights(x, like, opening=""):
        def piece(line, c):
            i = max(i for i, s in enumerate(starts) if s <= line * LINE + like)
            src, dst, s = matrices[i]
            return _piece(src, dst, sem_w.at[s], x + (line * LINE + c - starts[i]))

        q0, q1 = [], []
        skew = (opening.count("1") - opening.count("0") + 2) // 4
        for c0, cut in ((0, (lines + 1) // 2 - skew), (2, lines // 2)):
            q0 += [piece(line, c) for c in (c0, c0 + 1) for line in range(cut)]
            q1 += [piece(line, c) for c in (c0, c0 + 1) for line in range(cut, lines)]
        return _Stream(q0, q1, opening=opening)

    st = weights(0, 0, RAMP)
    while st.pos < len(st.order):
        st.more(4)
        fence()
    small = [pltpu.make_async_copy(src, dst, sem_w.at[s])
             for src, dst, s in ((c_hbm, c_v, s_c), (x_hbm, x_v, s_x), (b1_hbm, b1_v, s_b1))]
    for copy in small:
        copy.start()
    edges = [4] + sorted({s % LINE for s in starts} - {0}) + [LINE]
    for x0, x1 in zip(edges, edges[1:]):
        lax.fori_loop(x0 // 4, x1 // 4, lambda i, _, like=x0: weights(i * 4, like).rest(), None)

    def kv_pieces(src, u):
        rows = PAIR // SUB
        row0, col0, slot = u % NPAIR * rows, window_start + u // NPAIR % passes * PIECE, u % NSLOT

        def piece(r):
            return lambda o, n: pltpu.make_async_copy(
                src.at[row0 + r, pl.ds(col0 + o, n)],
                kv_v.at[slot, pl.ds(o, n), pl.ds(r * SUB, SUB), :], sem_kv.at[slot])

        return [[piece(r) for r in range(parity, rows, 2)] for parity in range(2)]

    def kv_stream(src, u, before=None):
        q0, q1 = kv_pieces(src, u)
        left_over = [] if before is None else kv_pieces(before, u - 1)[0][-KV_LAG:]
        st = _Stream(left_over + q0[:-KV_LAG], q1, opening="1" * (KV_LAG - len(left_over)))
        st.more(2 * KV_LAG)
        return st

    row = lax.broadcasted_iota(jnp.int32, (8, PAIR), 0)
    col = lax.broadcasted_iota(jnp.int32, (8, PAIR), 1)
    own = jnp.logical_or(jnp.logical_and(row == 0, col < DH), jnp.logical_and(row == 1, col >= DH))

    def query(p):
        n = PAIR // LANE
        parts = [_dot(h1, _column(wq_v, H * DH // LANE, p * n + j, 0, D)) for j in range(n)]
        q_s[p] = jnp.where(own, jnp.concatenate(parts, axis=1), 0.0)

    def scores(u, st):
        p, h, slot = u % NPAIR, u // NPAIR, u % NSLOT
        _wait_all(kv_v.at[slot], sem_kv.at[slot])
        q = q_s[p].astype(BF16)
        m = m_s[p]
        for c in range(PIECE):
            s = _dot(q, kv_v[slot, c]) * DH ** -0.5
            s_s[p, h * PIECE + c] = s
            m = jnp.maximum(m, s)
            st.more(4)
        m_s[p] = m

    def values(u, st=None):
        p, h, slot = u % NPAIR, u // NPAIR - passes, u % NSLOT
        _wait_all(kv_v.at[slot], sem_kv.at[slot])
        m = jnp.max(m_s[p], axis=-1, keepdims=True)
        l, acc = l_s[p], acc_s[p]
        for c in range(PIECE):
            e = jnp.exp(s_s[p, h * PIECE + c] - m)
            l += e
            acc += _dot_t(e.astype(BF16), kv_v[slot, c])
            if st is not None:
                st.more(4)
        l_s[p], acc_s[p] = l, acc

    def project(p):
        o = jnp.where(own, acc_s[p] / jnp.sum(l_s[p], axis=-1, keepdims=True), 0.0).astype(BF16)
        return jnp.concatenate([_dot(o, _column(wo_v, nd, j, p * PAIR, PAIR)) for j in range(nd)], axis=1)

    kv_stream(k_hbm, 0).rest()
    st = kv_stream(k_hbm, 1, k_hbm)
    st.upto(24)
    for copy in small:
        copy.wait()
    for _, buf, s in matrices:
        if s != s_w1:
            _wait_all(buf, sem_w.at[s])
    cf = c_v[...].astype(F32)
    silu_c = jnp.broadcast_to(cf * jax.nn.sigmoid(cf), (8, D)).astype(BF16)

    def modulation(i):
        for j in range(nd):
            mod_s[i, :, j * LANE:(j + 1) * LANE] = _dot(silu_c, _column(wmod_v, 6 * nd, i * nd + j, 0, D))

    modulation(0)
    modulation(1)
    st.rest()
    fence()
    x0 = jnp.broadcast_to(x_v[...].astype(F32), (8, D))
    h1 = (_layernorm(x0) * (1.0 + mod_s[1]) + mod_s[0]).astype(BF16)
    m_s[...] = jnp.full(m_s.shape, -jnp.inf, F32)
    for ref in (l_s, acc_s, att_s):
        ref[...] = jnp.zeros(ref.shape, F32)
    query(0)

    def k_loop(u0, u1, extra=None):
        def body(u, _):
            st = kv_stream(k_hbm, u, k_hbm)
            scores(u - 2, st)
            if extra is not None:
                fence()
                extra(u)
            st.rest()

        lax.fori_loop(u0, u1, body, None)

    k_loop(2, NPAIR + 1, lambda u: query(u - 1))
    k_loop(NPAIR + 1, NPAIR + 5, lambda u: modulation(u - NPAIR + 1))
    k_loop(NPAIR + 5, nu)
    for u, before in ((nu, k_hbm), (nu + 1, v_hbm)):
        st = kv_stream(v_hbm, u, before)
        scores(u - 2, st)
        st.rest()

    def v_body(final, u, _):
        st = kv_stream(v_hbm, u, v_hbm)
        if final:
            att_s[...] += project((u - 3) % NPAIR)
        values(u - 2, st)
        st.rest()

    last = 2 * nu - 1
    lax.fori_loop(nu + 2, last - NPAIR + 4, functools.partial(v_body, False), None)
    lax.fori_loop(last - NPAIR + 4, last + 1, functools.partial(v_body, True), None)

    late = [_piece(w1_hbm, w1_v, sem_w.at[s_w1], i) for i in range(W1_EARLY, w1_hbm.shape[0] // PIECE)]
    queues = kv_pieces(v_hbm, last)[0][-KV_LAG:] + late[:(len(late) - KV_LAG) // 2], late[(len(late) - KV_LAG) // 2:]
    for i, (queue, ranges) in enumerate(W2_MXU + W2_VPU):
        order = sorted((k - a, k) for a, b in ranges for k in range(a, b))
        queues[queue].extend(_piece(w2_hbm, w2_v, sem_w.at[s_w2 + i], k) for _, k in order)
    st = _Stream(*queues, parts=1)
    st.more(2 * KV_LAG)
    fence()
    st.upto(TAIL[0])
    values(last - 1)
    fence()
    st.upto(TAIL[1])
    values(last)
    fence()
    st.upto(TAIL[2])
    fence()

    att = att_s[...] + project(NPAIR - 3) + project(NPAIR - 2) + project(NPAIR - 1)
    x1 = x0 + mod_s[2] * jnp.broadcast_to(jnp.sum(att, axis=0, keepdims=True), (8, D))
    h2 = (_layernorm(x1) * (1.0 + mod_s[4]) + mod_s[3]).astype(BF16)
    b1 = b1_v[...].astype(F32)
    st.upto(TAIL[3])
    _wait_all(w1_v, sem_w.at[s_w1])
    up = [jnp.broadcast_to(b1[j:j + 1, :], (8, LANE)) + _dot(h2, _column(w1_v, nf, j, 0, D)) for j in range(nf)]
    act = _mish(jnp.concatenate(up, axis=1)).astype(BF16)
    fence()
    st.rest()

    tiles = [t for _, ranges in W2_VPU for a, b in ranges for t in range(a * PIECE, b * PIECE)]
    act_t = {j: jnp.broadcast_to(act[0:1, j * LANE:(j + 1) * LANE].astype(F32), (LANE, LANE)).T
             for j in sorted({t // nd * SUB // LANE for t in tiles})}
    factor = {}
    for t in tiles:
        r, j = t // nd * SUB, t % nd
        factor[t] = act_t[r // LANE][r % LANE:r % LANE + SUB] * mod_s[5, :, j * LANE:(j + 1) * LANE]

    def arrived(i, ranges):
        for a, b in ranges:
            _wait_all(w2_v.at[pl.ds(a * PIECE, (b - a) * PIECE)], sem_w.at[s_w2 + i])
        return [(a * PIECE, b * PIECE) for a, b in ranges]

    y = jnp.zeros((8, D), F32)
    for i, (_, ranges) in enumerate(W2_MXU):
        for t0, t1 in arrived(i, ranges):
            r0, r1 = t0 // nd * SUB, t1 // nd * SUB
            y += jnp.concatenate([_dot(act[:, r0:r1], _column(w2_v, nd, j, r0, r1 - r0)) for j in range(nd)], axis=1)
    out = jnp.where(lax.broadcasted_iota(jnp.int32, (8, D), 0) == 0, x1 + mod_s[5] * y, 0.0)
    out = [out[:, j * LANE:(j + 1) * LANE] for j in range(nd)]
    for i, (_, ranges) in enumerate(W2_VPU):
        for t0, t1 in arrived(len(W2_MXU) + i, ranges):
            for t in range(t0, t1):
                out[t % nd] += w2_v[t].astype(F32) * factor[t]
    o_ref[...] = jnp.sum(jnp.concatenate(out, axis=1), axis=0, keepdims=True).astype(o_ref.dtype)


def _tiles(a):
    r, c = a.shape
    return a.reshape(r // SUB, SUB, c // LANE, LANE).transpose(0, 2, 1, 3)


@jax.jit
def pallas_adaLN_cond__sliding_block_cached__dense_activation_mish__decode_kernel(
    A_x: jax.Array,
    A_k_cache: jax.Array,
    A_v_cache: jax.Array,
    A_wq: jax.Array,
    A_wo: jax.Array,
    B_x: jax.Array,
    B_w1: jax.Array,
    B_b1: jax.Array,
    B_w2: jax.Array,
    c: jax.Array,
    w_mod: jax.Array,
):
    del B_x
    sk = A_k_cache.shape[2]
    nc = min(4096, max(256, sk // 4)) // LANE
    kt, vt = (_tiles(jnp.swapaxes(a, 2, 3).reshape(H * DH, sk)) for a in (A_k_cache, A_v_cache))
    wmod, wq, wo, w1, w2 = (_tiles(a).reshape(-1, SUB, LANE) for a in (w_mod, A_wq, A_wo, B_w1, B_w2))
    out = pl.pallas_call(
        _kernel,
        out_shape=jax.ShapeDtypeStruct((1, D), A_x.dtype),
        in_specs=[pl.BlockSpec(memory_space=pltpu.HBM)] * 10,
        out_specs=pl.BlockSpec(memory_space=pltpu.VMEM),
        scratch_shapes=[
            pltpu.VMEM((1, D), BF16),
            pltpu.VMEM((1, D), BF16),
            pltpu.VMEM((F // LANE, LANE), BF16),
            *(pltpu.VMEM(a.shape, BF16) for a in (wmod, wq, wo, w1, w2)),
            pltpu.VMEM((NSLOT, PIECE, PAIR, LANE), BF16),
            pltpu.VMEM((6, 8, D), F32),
            pltpu.VMEM((NPAIR, 8, PAIR), F32),
            pltpu.VMEM((NPAIR, nc, 8, LANE), F32),
            pltpu.VMEM((NPAIR, 8, LANE), F32),
            pltpu.VMEM((NPAIR, 8, LANE), F32),
            pltpu.VMEM((NPAIR, 8, PAIR), F32),
            pltpu.VMEM((8, D), F32),
            pltpu.SemaphoreType.DMA((7 + len(W2_MXU + W2_VPU),)),
            pltpu.SemaphoreType.DMA((NSLOT,)),
            pltpu.SemaphoreType.REGULAR,
        ],
        compiler_params=pltpu.CompilerParams(
            vmem_limit_bytes=64 * 2**20,
            disable_semaphore_checks=True,
            disable_bounds_checks=True,
        ),
        name="adaln_attn_mlp_decode",
    )(A_x.reshape(1, D), kt, vt, wq, wo, w1, B_b1.reshape(F // LANE, LANE), w2, c, wmod)
    return out.reshape(A_x.shape)
```

```python
import functools

import jax
import jax.numpy as jnp
from jax import lax
import jax.experimental.pallas as pl
import jax.experimental.pallas.tpu as pltpu

D = 640
H = 32
DH = 192
F = 1536
PAIR = 2 * DH
NPAIR = H // 2
SUB, LANE = 8, 128
F32 = jnp.float32
BF16 = jnp.bfloat16

PIECE = 8
NSLOT = 4
KV_LAG = 4
LINE = 64
W1_EARLY = ((0, 20), (32, 56), (64, 84), (96, 116))
RAMP = "10111" * 5
W2_MXU = ((0, ((0, 20), (40, 60))), (1, ((60, 80), (100, 110))), (0, ((20, 40),)), (1, ((110, 120), (80, 85))))
W2_VPU = ((1, ((85, 92),)), (1, ((92, 97),)), (1, ((97, 99),)), (1, ((99, 100),)))
TAIL = (40, 80, 120, 150)


def _layernorm(x, eps=1e-5):
    m = jnp.mean(x, axis=-1, keepdims=True)
    d = x - m
    v = jnp.mean(d * d, axis=-1, keepdims=True)
    return d / jnp.sqrt(v + eps)


def _mish(u):
    softplus = jnp.log1p(jnp.exp(-jnp.abs(u))) + jnp.where(u > 0, u, 0.0)
    return u * jnp.tanh(softplus)


def _dot(a, b):
    return jnp.dot(a, b, preferred_element_type=F32)


def _dot_t(a, b):
    return lax.dot_general(a, b, (((1,), (1,)), ((), ())), preferred_element_type=F32)


def _column(buf, ncol, j, row0, nrow):
    t0 = row0 // SUB * ncol + j
    return jnp.stack([buf[t0 + r * ncol] for r in range(nrow // SUB)]).reshape(nrow, LANE)


def _piece(src, dst, sem, i):
    return lambda o, n: pltpu.make_async_copy(src.at[pl.ds(i * PIECE + o, n)], dst.at[pl.ds(i * PIECE + o, n)], sem)


def _wait_all(buf, sem):
    pltpu.make_async_copy(buf, buf, sem).wait()


class _Stream:
    def __init__(self, q0, q1, parts=2, opening=""):
        lists, pos = (q0, q1), [0, 0]
        self.order = []
        for queue in map(int, opening):
            self.order.append((lists[queue][pos[queue]], queue))
            pos[queue] += 1
        while len(self.order) < len(q0) + len(q1):
            for queue in (0, 1):
                self.order += [(piece, queue) for piece in lists[queue][pos[queue]:pos[queue] + 2]]
                pos[queue] += 2
        self.parts = parts
        self.pos = 0

    def more(self, n):
        for piece, queue in self.order[self.pos:self.pos + n]:
            size = PIECE // self.parts if queue else PIECE
            for o in range(0, PIECE, size):
                piece(o, size).start(priority=queue)
        self.pos += n

    def upto(self, n):
        self.more(max(n - self.pos, 0))

    def rest(self):
        self.upto(len(self.order))


def _kernel(x_hbm, k_hbm, v_hbm, wq_hbm, wo_hbm, w1_hbm, b1_hbm, w2_hbm, c_hbm, wmod_hbm, o_ref,
            x_v, c_v, b1_v, wmod_v, wq_v, wo_v, w1_v, w2_v, kv_v,
            mod_s, q_s, s_s, m_s, l_s, acc_s, att_s, sem_w, sem_kv, sem_fence):
    passes = s_s.shape[1] // PIECE
    window_start = k_hbm.shape[1] - passes * PIECE
    nu = passes * NPAIR
    nd, nf = D // LANE, F // LANE
    s_c, s_x, s_b1, s_wmod, s_wq, s_wo, s_w1, s_w2 = range(8)

    def fence():
        pl.semaphore_signal(sem_fence, 1)
        pl.semaphore_wait(sem_fence, 1)

    runs = [(src, dst, s, a, b)
            for src, dst, s in ((wmod_hbm, wmod_v, s_wmod), (w1_hbm, w1_v, s_w1), (wo_hbm, wo_v, s_wo), (wq_hbm, wq_v, s_wq))
            for a, b in (W1_EARLY if s == s_w1 else ((0, src.shape[0] // PIECE),))]
    starts = [0]
    for *_, a, b in runs:
        starts.append(starts[-1] + b - a)
    lines = starts[-1] // LINE
    assert lines * LINE == starts[-1] and all(s % 4 == 0 for s in starts)

    def weights(x, like, opening=""):
        def piece(line, c):
            i = max(i for i, s in enumerate(starts) if s <= line * LINE + like)
            src, dst, s, a, _ = runs[i]
            return _piece(src, dst, sem_w.at[s], x + (line * LINE + c - starts[i] + a))

        q0, q1 = [], []
        skew = (opening.count("1") - opening.count("0") + 2) // 4
        for c0, cut in ((0, (lines + 1) // 2 - skew), (2, lines // 2)):
            q0 += [piece(line, c) for c in (c0, c0 + 1) for line in range(cut)]
            q1 += [piece(line, c) for c in (c0, c0 + 1) for line in range(cut, lines)]
        return _Stream(q0, q1, opening=opening)

    st = weights(0, 0, RAMP)
    while st.pos < len(st.order):
        st.more(4)
        fence()
    small = [pltpu.make_async_copy(src, dst, sem_w.at[s])
             for src, dst, s in ((c_hbm, c_v, s_c), (x_hbm, x_v, s_x), (b1_hbm, b1_v, s_b1))]
    for copy in small:
        copy.start()
    edges = [4] + sorted({s % LINE for s in starts} - {0}) + [LINE]
    for x0, x1 in zip(edges, edges[1:]):
        lax.fori_loop(x0 // 4, x1 // 4, lambda i, _, like=x0: weights(i * 4, like).rest(), None)

    def kv_pieces(src, u):
        rows = PAIR // SUB
        row0, col0, slot = u % NPAIR * rows, window_start + u // NPAIR % passes * PIECE, u % NSLOT

        def piece(r):
            return lambda o, n: pltpu.make_async_copy(
                src.at[row0 + r, pl.ds(col0 + o, n)],
                kv_v.at[slot, pl.ds(o, n), pl.ds(r * SUB, SUB), :], sem_kv.at[slot])

        return [[piece(r) for r in range(parity, rows, 2)] for parity in range(2)]

    def kv_stream(src, u, before=None):
        q0, q1 = kv_pieces(src, u)
        left_over = [] if before is None else kv_pieces(before, u - 1)[0][-KV_LAG:]
        st = _Stream(left_over + q0[:-KV_LAG], q1, opening="1" * (KV_LAG - len(left_over)))
        st.more(2 * KV_LAG)
        return st

    row = lax.broadcasted_iota(jnp.int32, (8, PAIR), 0)
    col = lax.broadcasted_iota(jnp.int32, (8, PAIR), 1)
    own = jnp.logical_or(jnp.logical_and(row == 0, col < DH), jnp.logical_and(row == 1, col >= DH))

    def query(p):
        n = PAIR // LANE
        parts = [_dot(h1, _column(wq_v, H * DH // LANE, p * n + j, 0, D)) for j in range(n)]
        q_s[p] = jnp.where(own, jnp.concatenate(parts, axis=1), 0.0)

    def scores(u, st):
        p, h, slot = u % NPAIR, u // NPAIR, u % NSLOT
        _wait_all(kv_v.at[slot], sem_kv.at[slot])
        q = q_s[p].astype(BF16)
        m = m_s[p]
        for c in range(PIECE):
            s = _dot(q, kv_v[slot, c]) * DH ** -0.5
            s_s[p, h * PIECE + c] = s
            m = jnp.maximum(m, s)
            st.more(4)
        m_s[p] = m

    def values(u, st=None):
        p, h, slot = u % NPAIR, u // NPAIR - passes, u % NSLOT
        _wait_all(kv_v.at[slot], sem_kv.at[slot])
        m = jnp.max(m_s[p], axis=-1, keepdims=True)
        l, acc = l_s[p], acc_s[p]
        for c in range(PIECE):
            e = jnp.exp(s_s[p, h * PIECE + c] - m)
            l += e
            acc += _dot_t(e.astype(BF16), kv_v[slot, c])
            if st is not None:
                st.more(4)
        l_s[p], acc_s[p] = l, acc

    def project(p):
        o = jnp.where(own, acc_s[p] / jnp.sum(l_s[p], axis=-1, keepdims=True), 0.0).astype(BF16)
        return jnp.concatenate([_dot(o, _column(wo_v, nd, j, p * PAIR, PAIR)) for j in range(nd)], axis=1)

    kv_stream(k_hbm, 0).rest()
    st = kv_stream(k_hbm, 1, k_hbm)
    st.upto(24)
    for copy in small:
        copy.wait()
    for buf, s in ((wmod_v, s_wmod), (wo_v, s_wo), (wq_v, s_wq)):
        _wait_all(buf, sem_w.at[s])
    cf = c_v[...].astype(F32)
    silu_c = jnp.broadcast_to(cf * jax.nn.sigmoid(cf), (8, D)).astype(BF16)

    def modulation(i):
        for j in range(nd):
            mod_s[i, :, j * LANE:(j + 1) * LANE] = _dot(silu_c, _column(wmod_v, 6 * nd, i * nd + j, 0, D))

    modulation(0)
    modulation(1)
    st.rest()
    fence()
    x0 = jnp.broadcast_to(x_v[...].astype(F32), (8, D))
    h1 = (_layernorm(x0) * (1.0 + mod_s[1]) + mod_s[0]).astype(BF16)
    m_s[...] = jnp.full(m_s.shape, -jnp.inf, F32)
    for ref in (l_s, acc_s, att_s):
        ref[...] = jnp.zeros(ref.shape, F32)
    query(0)

    def k_loop(u0, u1, extra=None):
        def body(u, _):
            st = kv_stream(k_hbm, u, k_hbm)
            scores(u - 2, st)
            if extra is not None:
                fence()
                extra(u)
            st.rest()

        lax.fori_loop(u0, u1, body, None)

    k_loop(2, NPAIR + 1, lambda u: query(u - 1))
    k_loop(NPAIR + 1, NPAIR + 5, lambda u: modulation(u - NPAIR + 1))
    k_loop(NPAIR + 5, nu)
    for u, before in ((nu, k_hbm), (nu + 1, v_hbm)):
        st = kv_stream(v_hbm, u, before)
        scores(u - 2, st)
        st.rest()

    def v_body(final, u, _):
        st = kv_stream(v_hbm, u, v_hbm)
        if final:
            att_s[...] += project((u - 3) % NPAIR)
        values(u - 2, st)
        st.rest()

    last = 2 * nu - 1
    lax.fori_loop(nu + 2, last - NPAIR + 4, functools.partial(v_body, False), None)
    lax.fori_loop(last - NPAIR + 4, last + 1, functools.partial(v_body, True), None)

    gaps = zip([b for _, b in W1_EARLY], [a for a, _ in W1_EARLY[1:]] + [w1_hbm.shape[0] // PIECE])
    late = [_piece(w1_hbm, w1_v, sem_w.at[s_w1], k) for _, k in sorted((k - a, k) for a, b in gaps for k in range(a, b))]
    late = kv_pieces(v_hbm, last)[0][-KV_LAG:] + late
    queues = late[:len(late) // 2], late[len(late) // 2:]
    for i, (queue, ranges) in enumerate(W2_MXU + W2_VPU):
        order = sorted((k - a, k) for a, b in ranges for k in range(a, b))
        queues[queue].extend(_piece(w2_hbm, w2_v, sem_w.at[s_w2 + i], k) for _, k in order)
    st = _Stream(*queues, parts=1)
    st.more(2 * KV_LAG)
    fence()
    st.upto(TAIL[0])
    values(last - 1)
    fence()
    st.upto(TAIL[1])
    values(last)
    fence()
    st.upto(TAIL[2])
    fence()

    att = att_s[...] + project(NPAIR - 3) + project(NPAIR - 2) + project(NPAIR - 1)
    x1 = x0 + mod_s[2] * jnp.broadcast_to(jnp.sum(att, axis=0, keepdims=True), (8, D))
    h2 = (_layernorm(x1) * (1.0 + mod_s[4]) + mod_s[3]).astype(BF16)
    b1 = b1_v[...].astype(F32)
    st.upto(TAIL[3])
    _wait_all(w1_v, sem_w.at[s_w1])
    up = [jnp.broadcast_to(b1[j:j + 1, :], (8, LANE)) + _dot(h2, _column(w1_v, nf, j, 0, D)) for j in range(nf)]
    act = _mish(jnp.concatenate(up, axis=1)).astype(BF16)
    fence()
    st.rest()

    tiles = [t for _, ranges in W2_VPU for a, b in ranges for t in range(a * PIECE, b * PIECE)]
    act_t = {j: jnp.broadcast_to(act[0:1, j * LANE:(j + 1) * LANE].astype(F32), (LANE, LANE)).T
             for j in sorted({t // nd * SUB // LANE for t in tiles})}
    factor = {}
    for t in tiles:
        r, j = t // nd * SUB, t % nd
        factor[t] = act_t[r // LANE][r % LANE:r % LANE + SUB] * mod_s[5, :, j * LANE:(j + 1) * LANE]

    def arrived(i, ranges):
        for a, b in ranges:
            _wait_all(w2_v.at[pl.ds(a * PIECE, (b - a) * PIECE)], sem_w.at[s_w2 + i])
        return [(a * PIECE, b * PIECE) for a, b in ranges]

    y = jnp.zeros((8, D), F32)
    for i, (_, ranges) in enumerate(W2_MXU):
        for t0, t1 in arrived(i, ranges):
            r0, r1 = t0 // nd * SUB, t1 // nd * SUB
            y += jnp.concatenate([_dot(act[:, r0:r1], _column(w2_v, nd, j, r0, r1 - r0)) for j in range(nd)], axis=1)
    out = jnp.where(lax.broadcasted_iota(jnp.int32, (8, D), 0) == 0, x1 + mod_s[5] * y, 0.0)
    out = [out[:, j * LANE:(j + 1) * LANE] for j in range(nd)]
    for i, (_, ranges) in enumerate(W2_VPU):
        for t0, t1 in arrived(len(W2_MXU) + i, ranges):
            for t in range(t0, t1):
                out[t % nd] += w2_v[t].astype(F32) * factor[t]
    o_ref[...] = jnp.sum(jnp.concatenate(out, axis=1), axis=0, keepdims=True).astype(o_ref.dtype)


def _tiles(a):
    r, c = a.shape
    return a.reshape(r // SUB, SUB, c // LANE, LANE).transpose(0, 2, 1, 3)


@jax.jit
def pallas_adaLN_cond__sliding_block_cached__dense_activation_mish__decode_kernel(
    A_x: jax.Array,
    A_k_cache: jax.Array,
    A_v_cache: jax.Array,
    A_wq: jax.Array,
    A_wo: jax.Array,
    B_x: jax.Array,
    B_w1: jax.Array,
    B_b1: jax.Array,
    B_w2: jax.Array,
    c: jax.Array,
    w_mod: jax.Array,
):
    del B_x
    sk = A_k_cache.shape[2]
    nc = min(4096, max(256, sk // 4)) // LANE
    kt, vt = (_tiles(jnp.swapaxes(a, 2, 3).reshape(H * DH, sk)) for a in (A_k_cache, A_v_cache))
    wmod, wq, wo, w1, w2 = (_tiles(a).reshape(-1, SUB, LANE) for a in (w_mod, A_wq, A_wo, B_w1, B_w2))
    out = pl.pallas_call(
        _kernel,
        out_shape=jax.ShapeDtypeStruct((1, D), A_x.dtype),
        in_specs=[pl.BlockSpec(memory_space=pltpu.HBM)] * 10,
        out_specs=pl.BlockSpec(memory_space=pltpu.VMEM),
        scratch_shapes=[
            pltpu.VMEM((1, D), BF16),
            pltpu.VMEM((1, D), BF16),
            pltpu.VMEM((F // LANE, LANE), BF16),
            *(pltpu.VMEM(a.shape, BF16) for a in (wmod, wq, wo, w1, w2)),
            pltpu.VMEM((NSLOT, PIECE, PAIR, LANE), BF16),
            pltpu.VMEM((6, 8, D), F32),
            pltpu.VMEM((NPAIR, 8, PAIR), F32),
            pltpu.VMEM((NPAIR, nc, 8, LANE), F32),
            pltpu.VMEM((NPAIR, 8, LANE), F32),
            pltpu.VMEM((NPAIR, 8, LANE), F32),
            pltpu.VMEM((NPAIR, 8, PAIR), F32),
            pltpu.VMEM((8, D), F32),
            pltpu.SemaphoreType.DMA((7 + len(W2_MXU + W2_VPU),)),
            pltpu.SemaphoreType.DMA((NSLOT,)),
            pltpu.SemaphoreType.REGULAR,
        ],
        compiler_params=pltpu.CompilerParams(
            vmem_limit_bytes=64 * 2**20,
            disable_semaphore_checks=True,
            disable_bounds_checks=True,
        ),
        name="adaln_attn_mlp_decode",
    )(A_x.reshape(1, D), kt, vt, wq, wo, w1, B_b1.reshape(F // LANE, LANE), w2, c, wmod)
    return out.reshape(A_x.shape)
```
